```python
import jax
import jax.numpy as jnp

def _softmax(x, axis=-1):
    return jax.nn.softmax(x, axis=axis)
def _gelu(x):
    return jax.nn.gelu(x, approximate=True)
def _silu(x):
    return jax.nn.silu(x)
def _sigmoid(x):
    return jax.nn.sigmoid(x)
def _layernorm(x, axis=-1, eps=1e-5):
    m = jnp.mean(x, axis=axis, keepdims=True)
    v = jnp.var(x, axis=axis, keepdims=True)
    return (x - m) / jnp.sqrt(v + eps)
def _scatter_add(tgt, idx, src, axis=0):
    return tgt.at[idx].add(src)
def _segment_sum(src, seg, n):
    return jax.ops.segment_sum(src, seg, n)
class _Rng:
    def __init__(self, key):
        self._k = key
    def _next(self):
        self._k, sub = jax.random.split(self._k)
        return sub
    def normal(self, shape):
        return jax.random.normal(self._next(), shape, dtype=jnp.bfloat16)
    def randint(self, lo, hi, shape):
        return jax.random.randint(self._next(), shape, lo, hi, dtype=jnp.int32)
    def uniform(self, shape, lo=0.0, hi=1.0):
        return jax.random.uniform(self._next(), shape, jnp.bfloat16, lo, hi)
    def permutation(self, n):
        return jax.random.permutation(self._next(), n)


kernel_name = 'gated_mix__ssm_conv_h3__sliding_local_dilated__prompt'

def setup_inputs():
    _rng = _Rng(jax.random.key(int.from_bytes(__import__("os").urandom(4), "little")))
    _w = (lambda a: (lambda t: t.astype(jnp.bfloat16) if jnp.issubdtype(t.dtype, jnp.floating) else t)(jnp.asarray(a)))
    def _A_setup():
        B, S, D = 1, 2048, 640
        ks = 4
        return {
            "q": _w((lambda *s: _rng.normal(s) * 0.05)(B, S, D)),
            "k": _w((lambda *s: _rng.normal(s) * 0.05)(B, S, D)),
            "v": _w((lambda *s: _rng.normal(s) * 0.05)(B, S, D)),
            "shift_k": _w((lambda *s: _rng.normal(s) * 0.05)(D, ks) * 0.5),
            "ssm_k": _w((lambda *s: _rng.normal(s) * 0.05)(D, S) * (1.0 / S ** 0.5)),
            "ssm_D": _w((lambda *s: _rng.normal(s) * 0.05)(D)),
        }
    _A_in = _A_setup()

    def _B_setup():
        B, S, D = 1, 2048, 640
        return {
            "x": _w((lambda *s: _rng.normal(s) * 0.05)(B, S, D)),
            "wqkv": _w((lambda *s: _rng.normal(s) * 0.05)(D, 3 * D)),
            "wo": _w((lambda *s: _rng.normal(s) * 0.05)(D, D)),
        }
    _B_in = _B_setup()

    return {
        "A_q": _A_in["q"],
        "A_k": _A_in["k"],
        "A_v": _A_in["v"],
        "A_shift_k": _A_in["shift_k"],
        "A_ssm_k": _A_in["ssm_k"],
        "A_ssm_D": _A_in["ssm_D"],
        "B_x": _B_in["x"],
        "B_wqkv": _B_in["wqkv"],
        "B_wo": _B_in["wo"],
        "gate_w": _w((lambda *s: _rng.normal(s) * 0.05)(640)),
    }

def reference(A_q, A_k, A_v, A_shift_k, A_ssm_k, A_ssm_D, B_x, B_wqkv, B_wo, gate_w):
    def _A_ref(q, k, v, shift_k, ssm_k, ssm_D):
        B, S, D = q.shape
        ks = shift_k.shape[-1]
        k_pad = jnp.pad(k, ((0, 0), (ks - 1, 0), (0, 0)))
        k_shift = jnp.zeros_like(k)
        for t in range(ks):
            k_shift = k_shift + k_pad[:, t:t + S, :] * shift_k[:, ks - 1 - t][None, None, :]
        kv = k_shift * v
        L = 2 * S
        kv_pad = jnp.pad(kv, ((0, 0), (0, S), (0, 0)))
        kf_pad = jnp.pad(ssm_k, ((0, 0), (0, S)))
        kv_f = (lambda x, axes=(-2,-1): jnp.fft.rfft2(x.astype(jnp.float32), axes=axes))(kv_pad[:, None, :, :], axes=(1, 2))
        kf_f = (lambda x, axes=(-2,-1): jnp.fft.rfft2(x.astype(jnp.float32), axes=axes))(kf_pad[:, None, :], axes=(1, 2))
        kf_f = (lambda x, *d: x.transpose(*d))(kf_f, 1, 2, 0)
        y_f = kv_f * kf_f[None, :, :, :]
        y = (lambda x, s, axes=(-2,-1): jnp.fft.irfft2(x, s=s, axes=axes).astype(jnp.bfloat16))(y_f, (1, L), axes=(1, 2))[:, 0, :S, :]
        y = y + kv * ssm_D[None, None, :]
        return q * y

    def _B_ref(x, wqkv, wo):
        B, S, D = x.shape
        H = 32; Dh = D // H
        W, dil = 8, 2
        qkv = (lambda x, *d: x.transpose(*d))((x @ wqkv).reshape(B, S, 3, H, Dh), 2, 0, 3, 1, 4)
        q, k, v = qkv[0], qkv[1], qkv[2]
        scale = Dh ** -0.5
        pos = jnp.arange(S)
        off = jnp.arange(W) * dil
        idx = pos[:, None] - off[None, :]
        mask = idx >= 0
        idx_c = jnp.where(mask, idx, 0).reshape(-1)
        kg = k[:, :, idx_c, :].reshape(B, H, S, W, Dh)
        vg = v[:, :, idx_c, :].reshape(B, H, S, W, Dh)
        logits = jnp.einsum("bhsd,bhswd->bhsw", q, kg) * scale
        logits = jnp.where(mask[None, None, :, :], logits, -1e9)
        attn = _softmax(logits, axis=-1)
        o = jnp.einsum("bhsw,bhswd->bhsd", attn, vg)
        return (lambda x, *d: x.transpose(*d))(o, 0, 2, 1, 3).reshape(B, S, D) @ wo

    x = A_q
    g = _sigmoid((x * gate_w).sum(-1, keepdims=True))
    a = _A_ref(x, A_k, A_v, A_shift_k, A_ssm_k, A_ssm_D)
    b = _B_ref(x, B_wqkv, B_wo)
    return g * a + (1 - g) * b
```

```python
import functools

import jax
import jax.numpy as jnp
import numpy as np
import jax.experimental.pallas as pl
import jax.experimental.pallas.tpu as pltpu

S, D = 2048, 640
H, DH, W, DIL = 32, 20, 8, 2
KS = 4
NC = D // 128
T = 256
NT = S // T
HALO = 16
L, PC = 1024, 512
NP = S // PC
LOG2E = 1.4426950408889634
QSCALE = (DH ** -0.5) * LOG2E
F32, BF16 = jnp.float32, jnp.bfloat16


def _dft_tables():
    rho = np.arange(128)
    k1 = np.where(rho < 64, 2 * rho, 2 * (rho - 64) + 1)
    s1 = np.arange(128)
    f = np.zeros((4, 256, 128), np.float64)
    for s2 in range(4):
        ph = ((2 * k1[:, None] + 1) * (4 * s1[None, :] + s2)) % (2 * L)
        th = 2 * np.pi * ph / (2 * L)
        f[s2, :128] = np.cos(th)
        f[s2, 128:] = -np.sin(th)
    g = f.transpose(0, 2, 1) * (2.0 / L)
    return f.astype(np.float32), g.astype(np.float32)


def _fft4(z):
    e0 = (z[0][0] + z[2][0], z[0][1] + z[2][1])
    e1 = (z[0][0] - z[2][0], z[0][1] - z[2][1])
    o0 = (z[1][0] + z[3][0], z[1][1] + z[3][1])
    o1 = (z[1][0] - z[3][0], z[1][1] - z[3][1])
    return [
        (e0[0] + o0[0], e0[1] + o0[1]),
        (e1[0] + o1[1], e1[1] - o1[0]),
        (e0[0] - o0[0], e0[1] - o0[1]),
        (e1[0] - o1[1], e1[1] + o1[0]),
    ]


def _ifft4(y):
    a = (y[0][0] + y[2][0], y[0][1] + y[2][1])
    b = (y[0][0] - y[2][0], y[0][1] - y[2][1])
    c = (y[1][0] + y[3][0], y[1][1] + y[3][1])
    d = (y[1][0] - y[3][0], y[1][1] - y[3][1])
    return [
        (a[0] + c[0], a[1] + c[1]),
        (b[0] - d[1], b[1] + d[0]),
        (a[0] - c[0], a[1] - c[1]),
        (b[0] + d[1], b[1] - d[0]),
    ]


def _kernel(x_hbm, k_hbm, v_hbm, sk_hbm, h_hbm, dv_hbm, w_hbm, wo_hbm, gw_hbm,
            f_hbm, g_hbm, out_hbm,
            k_v, v_v, sk_v, h_v, dv_v, x_v, w_v, wo_v, gw_v, f_v, g_v,
            wt_s, wo_s, tmp_s, bq_s, bk_s, bv_s, o_s, b_s,
            kf_s, u_s, ht_s, z_s, vv_s, y_s, out_s, sems):
    nsem = [0]

    def dma(src, dst):
        cp = pltpu.make_async_copy(src, dst, sems.at[nsem[0]])
        nsem[0] += 1
        cp.start()
        return cp

    def x_dma(i):
        return dma(x_hbm.at[pl.ds(i * T, T), :], x_v.at[pl.ds(i * T, T), :])

    def a_dma(c):
        return [dma(k_hbm.at[:, pl.ds(c * 128, 128)], k_v.at[c]),
                dma(v_hbm.at[:, pl.ds(c * 128, 128)], v_v.at[c]),
                dma(h_hbm.at[pl.ds(c * 128, 128), :], h_v.at[c])]

    cp_w = [dma(w_hbm.at[:, pl.ds(0, D)], w_v.at[0])]
    cp_x = [x_dma(0)]
    cp_w += [dma(w_hbm.at[:, pl.ds(p * D, D)], w_v.at[p]) for p in (1, 2)]
    cp_small = [dma(sk_hbm, sk_v), dma(dv_hbm, dv_v), dma(gw_hbm, gw_v)]
    cp_f = dma(f_hbm, f_v)
    cp_a = [a_dma(0)]
    cp_wo = dma(wo_hbm, wo_v)
    cp_x.append(x_dma(1))
    cp_a.append(a_dma(1))
    cp_x.append(x_dma(2))
    cp_a.append(a_dma(2))
    cp_g = dma(g_hbm, g_v)
    cp_a.append(a_dma(3))
    cp_x.append(x_dma(3))
    cp_a.append(a_dma(4))
    cp_x += [x_dma(i) for i in range(4, NT)]

    def prep_w(p):
        for rc in range(NC):
            tmp_s[p, rc] = w_v[p, rc * 128:(rc + 1) * 128, :].astype(F32).T
        for rc in range(NC):
            for d in range(DH):
                wt_s[p * D + d * H:p * D + (d + 1) * H, rc * 128:(rc + 1) * 128] = (
                    tmp_s[p, rc, pl.ds(d, H, stride=DH), :].astype(BF16))

    def prep_wo():
        for cc in range(NC):
            tmp_s[3, cc] = wo_v[:, cc * 128:(cc + 1) * 128].astype(F32)
        for cc in range(NC):
            for d in range(DH):
                wo_s[d * H:(d + 1) * H, cc * 128:(cc + 1) * 128] = (
                    tmp_s[3, cc, pl.ds(d, H, stride=DH), :].astype(BF16))

    def proj(i):
        r0 = i * T
        qkv = jax.lax.dot_general(x_v[r0:r0 + T, :], wt_s[...], (((1,), (1,)), ((), ())),
                                  preferred_element_type=F32)
        for c in range(NC):
            bq_s[c, r0:r0 + T, :] = qkv[:, c * 128:(c + 1) * 128] * QSCALE
            bk_s[c, HALO + r0:HALO + r0 + T, :] = qkv[:, D + c * 128:D + (c + 1) * 128]
            bv_s[c, HALO + r0:HALO + r0 + T, :] = qkv[:, 2 * D + c * 128:2 * D + (c + 1) * 128]

    def attn(i):
        ch = 8
        for r in range(i * T, (i + 1) * T, ch):
            q = [bq_s[c, r:r + ch, :] for c in range(NC)]
            ls = []
            for w in range(W):
                o = HALO + r - DIL * w
                t = q[0] * bk_s[0, o:o + ch, :]
                for c in range(1, NC):
                    t = t + q[c] * bk_s[c, o:o + ch, :]
                t = t + pltpu.roll(t, 64, 1)
                t = t + pltpu.roll(t, 32, 1)
                if r < DIL * w:
                    row = jax.lax.broadcasted_iota(jnp.int32, (ch, 128), 0) + r
                    t = jnp.where(row >= DIL * w, t, -1e9 * LOG2E)
                ls.append(t)
            m = functools.reduce(jnp.maximum, ls)
            ps = [jnp.exp2(l - m) for l in ls]
            inv = 1.0 / functools.reduce(lambda a, b: a + b, ps)
            for c in range(NC):
                acc = ps[0] * bv_s[c, HALO + r:HALO + r + ch, :]
                for w in range(1, W):
                    o = HALO + r - DIL * w
                    acc = acc + ps[w] * bv_s[c, o:o + ch, :]
                o_s[r:r + ch, c * 128:(c + 1) * 128] = acc * inv

    def outp(i):
        r0 = i * T
        b_s[r0:r0 + T, :] = jnp.dot(o_s[r0:r0 + T, :].astype(BF16), wo_s[...],
                                    preferred_element_type=F32)

    def a1(c):
        cs = slice(c * 128, (c + 1) * 128)
        taps = [sk_v[j:j + 1, cs].astype(F32) for j in range(KS)]
        kf_s[c, 0:8, :] = jnp.zeros((8, 128), F32)
        rb = 64
        for r in range(0, S, rb):
            kf_s[c, 8 + r:8 + r + rb, :] = k_v[c, r:r + rb, :].astype(F32)
        for r in range(0, S, rb):
            ks = kf_s[c, 8 + r:8 + r + rb, :] * taps[0]
            for j in range(1, KS):
                ks = ks + kf_s[c, 8 + r - j:8 + r - j + rb, :] * taps[j]
            u_s[c, r:r + rb, :] = ks * v_v[c, r:r + rb, :].astype(F32)
        for j in range(NP):
            ht_s[c, j * PC:(j + 1) * PC, :] = h_v[c, :, j * PC:(j + 1) * PC].astype(F32).T
        for s2 in range(4):
            cols = [u_s[c, pl.ds(j * PC + s2, 128, stride=4), :].astype(BF16) for j in range(NP)]
            cols += [ht_s[c, pl.ds(j * PC + s2, 128, stride=4), :].astype(BF16) for j in range(NP)]
            z_s[c, s2] = jnp.dot(f_v[s2], jnp.concatenate(cols, axis=1), preferred_element_type=F32)

    def a2(c):
        ch = 8
        for r in range(0, 128, ch):
            def ld(piece):
                ls = slice(piece * 128, (piece + 1) * 128)
                return [(z_s[c, s2, r:r + ch, ls], z_s[c, s2, 128 + r:128 + r + ch, ls])
                        for s2 in range(4)]
            hh = [_fft4(ld(NP + a)) for a in range(NP)]
            gg = [hh[0]]
            for a in range(1, NP):
                if r < 64:
                    gg.append([(hh[a][k][0] - hh[a - 1][k][1], hh[a][k][1] + hh[a - 1][k][0])
                               for k in range(4)])
                else:
                    gg.append([(hh[a][k][0] + hh[a - 1][k][1], hh[a][k][1] - hh[a - 1][k][0])
                               for k in range(4)])
            uu = [_fft4(ld(b)) for b in range(NP)]
            for m in range(NP):
                ys = []
                for k in range(4):
                    re = im = None
                    for b in range(m + 1):
                        ur, ui = uu[b][k]
                        gr, gi = gg[m - b][k]
                        pr = ur * gr - ui * gi
                        pi = ur * gi + ui * gr
                        re = pr if re is None else re + pr
                        im = pi if im is None else im + pi
                    ys.append((re, im))
                vs = _ifft4(ys)
                ms = slice(m * 128, (m + 1) * 128)
                for s2 in range(4):
                    vv_s[c, s2, r:r + ch, ms] = vs[s2][0]
                    vv_s[c, s2, 128 + r:128 + r + ch, ms] = vs[s2][1]

    def a3(c):
        for s2 in range(4):
            res = jnp.dot(g_v[s2], vv_s[c, s2].astype(BF16), preferred_element_type=F32)
            for m in range(NP):
                y_s[c, pl.ds(m * PC + s2, 128, stride=4), :] = res[:, m * 128:(m + 1) * 128]

    out_cps = []

    def final(i):
        ch = 16
        gw = [gw_v[c * 128:(c + 1) * 128].astype(F32).reshape(1, 128) for c in range(NC)]
        dv = [dv_v[c * 128:(c + 1) * 128].astype(F32).reshape(1, 128) for c in range(NC)]
        for r in range(i * T, (i + 1) * T, ch):
            qf = [x_v[r:r + ch, c * 128:(c + 1) * 128].astype(F32) for c in range(NC)]
            z = qf[0] * gw[0]
            for c in range(1, NC):
                z = z + qf[c] * gw[c]
            g = jax.nn.sigmoid(jnp.sum(z, axis=1, keepdims=True))
            for c in range(NC):
                a = qf[c] * (y_s[c, r:r + ch, :] + u_s[c, r:r + ch, :] * dv[c])
                b = b_s[r:r + ch, c * 128:(c + 1) * 128]
                out_s[r:r + ch, c * 128:(c + 1) * 128] = (b + g * (a - b)).astype(BF16)
        out_cps.append(dma(out_s.at[pl.ds(i * T, T), :], out_hbm.at[pl.ds(i * T, T), :]))

    def wait(cps):
        for cp in cps:
            cp.wait()

    for c in range(NC):
        bk_s[c, 0:HALO, :] = jnp.zeros((HALO, 128), F32)
        bv_s[c, 0:HALO, :] = jnp.zeros((HALO, 128), F32)

    wait([cp_w[0], cp_x[0]])
    prep_w(0)
    wait(cp_w[1:])
    prep_w(1)
    prep_w(2)
    proj(0)
    wait([cp_wo, cp_x[1]] + cp_small + [cp_f] + cp_a[0])
    prep_wo()
    proj(1); a1(0); attn(0); outp(0)
    wait([cp_x[2]] + cp_a[1] + cp_a[2])
    proj(2); a1(1); a1(2); a2(0); attn(1); outp(1)
    wait([cp_x[3], cp_g] + cp_a[3] + cp_a[4])
    proj(3); a1(3); a1(4); a2(1); a2(2); a3(0); attn(2); outp(2)
    wait([cp_x[4]])
    proj(4); a2(3); a2(4); a3(1); a3(2); attn(3); outp(3)
    wait([cp_x[5]])
    proj(5); a3(3); a3(4); attn(4); outp(4)
    wait([cp_x[6]])
    proj(6); attn(5); outp(5)
    for i in range(0, 4):
        final(i)
    wait([cp_x[7]])
    proj(7); attn(6); outp(6)
    for i in range(4, 7):
        final(i)
    attn(7); outp(7); final(7)
    wait(out_cps)


@jax.jit
def pallas_gated_mix__ssm_conv_h3__sliding_local_dilated__prompt_kernel(
    A_q: jax.Array,
    A_k: jax.Array,
    A_v: jax.Array,
    A_shift_k: jax.Array,
    A_ssm_k: jax.Array,
    A_ssm_D: jax.Array,
    B_x: jax.Array,
    B_wqkv: jax.Array,
    B_wo: jax.Array,
    gate_w: jax.Array,
):
    f_np, g_np = _dft_tables()
    f_tab = jnp.asarray(f_np, dtype=BF16)
    g_tab = jnp.asarray(g_np, dtype=BF16)
    vm = pltpu.VMEM
    scratch = [
        vm((NC, S, 128), BF16),
        vm((NC, S, 128), BF16),
        vm((KS, D), BF16),
        vm((NC, 128, S), BF16),
        vm((D,), BF16),
        vm((S, D), BF16),
        vm((3, D, D), BF16),
        vm((D, D), BF16),
        vm((D,), BF16),
        vm((4, 256, 128), BF16),
        vm((4, 128, 256), BF16),
        vm((3 * D, D), BF16),
        vm((D, D), BF16),
        vm((4, NC, D, 128), F32),
        vm((NC, S, 128), F32),
        vm((NC, S + HALO, 128), F32),
        vm((NC, S + HALO, 128), F32),
        vm((S, D), F32),
        vm((S, D), F32),
        vm((NC, S + 8, 128), F32),
        vm((NC, S, 128), F32),
        vm((NC, S, 128), F32),
        vm((NC, 4, 256, 1024), F32),
        vm((NC, 4, 256, 512), F32),
        vm((NC, S, 128), F32),
        vm((S, D), BF16),
        pltpu.SemaphoreType.DMA((48,)),
    ]
    out = pl.pallas_call(
        _kernel,
        out_shape=jax.ShapeDtypeStruct((S, D), BF16),
        in_specs=[pl.BlockSpec(memory_space=pl.ANY)] * 11,
        out_specs=pl.BlockSpec(memory_space=pl.ANY),
        scratch_shapes=scratch,
        compiler_params=pltpu.CompilerParams(vmem_limit_bytes=126 * 1024 * 1024),
    )(A_q.reshape(S, D), A_k.reshape(S, D), A_v.reshape(S, D), A_shift_k.T, A_ssm_k, A_ssm_D,
      B_wqkv, B_wo, gate_w, f_tab, g_tab)
    return out.reshape(1, S, D)
```

```python
import functools

import jax
import jax.numpy as jnp
import numpy as np
import jax.experimental.pallas as pl
import jax.experimental.pallas.tpu as pltpu

S, D = 2048, 640
H, DH, W, DIL = 32, 20, 8, 2
KS = 4
NC = D // 128
T = 256
NT = S // T
HALO = 16
L, PC = 1024, 512
NP = S // PC
LOG2E = 1.4426950408889634
QSCALE = (DH ** -0.5) * LOG2E
F32, BF16, U32 = jnp.float32, jnp.bfloat16, jnp.uint32
import os
CFG = dict(SPAN=0.92, RATE=2.6, ATGAP=120, VERB=0, DYN=1, NS=128, NSF=128, NSI=128, LA=3, L2=1, LF=2, LK=1, LH=1, GLOBAL=1, ROT3=1, SEQ=1, FULL=1, KCH=1, RHS=1, PART='all', SCHED='A')
for _k in CFG:
    if _k in os.environ:
        CFG[_k] = type(CFG[_k])(os.environ[_k])


def _dft_tables():
    rho = np.arange(128)
    k1 = np.where(rho < 64, 2 * rho, 2 * (rho - 64) + 1)
    s1 = np.arange(128)
    f = np.zeros((4, 256, 128), np.float64)
    for s2 in range(4):
        ph = ((2 * k1[:, None] + 1) * (4 * s1[None, :] + s2)) % (2 * L)
        th = 2 * np.pi * ph / (2 * L)
        f[s2, :128] = np.cos(th)
        f[s2, 128:] = -np.sin(th)
    g = f.transpose(0, 2, 1) * (2.0 / L)
    g = g.reshape(4, 128, 2, 128).transpose(0, 1, 3, 2).reshape(4, 128, 256)
    return f.astype(np.float32), g.astype(np.float32)


def _fft4(z):
    e0 = (z[0][0] + z[2][0], z[0][1] + z[2][1])
    e1 = (z[0][0] - z[2][0], z[0][1] - z[2][1])
    o0 = (z[1][0] + z[3][0], z[1][1] + z[3][1])
    o1 = (z[1][0] - z[3][0], z[1][1] - z[3][1])
    return [
        (e0[0] + o0[0], e0[1] + o0[1]),
        (e1[0] + o1[1], e1[1] - o1[0]),
        (e0[0] - o0[0], e0[1] - o0[1]),
        (e1[0] - o1[1], e1[1] + o1[0]),
    ]


def _ifft4(y):
    a = (y[0][0] + y[2][0], y[0][1] + y[2][1])
    b = (y[0][0] - y[2][0], y[0][1] - y[2][1])
    c = (y[1][0] + y[3][0], y[1][1] + y[3][1])
    d = (y[1][0] - y[3][0], y[1][1] - y[3][1])
    return [
        (a[0] + c[0], a[1] + c[1]),
        (b[0] - d[1], b[1] + d[0]),
        (a[0] - c[0], a[1] - c[1]),
        (b[0] + d[1], b[1] - d[0]),
    ]


def _tree(xs, op):
    xs = list(xs)
    while len(xs) > 1:
        xs = [op(xs[i], xs[i + 1]) if i + 1 < len(xs) else xs[i] for i in range(0, len(xs), 2)]
    return xs[0]


def _add(a, b):
    return a + b


def _sum(xs):
    if CFG['SEQ']:
        return functools.reduce(_add, xs)
    return _tree(xs, _add)


def _pk(x):
    return pltpu.bitcast(x.astype(BF16), U32)


def _pk2(a, b):
    return pltpu.pack_elementwise([a, b], packed_dtype=BF16)


def _up(x):
    return pltpu.bitcast(x, BF16)


def _pack_table(t):
    u = t.astype(jnp.bfloat16).view(np.uint16).astype(np.uint32)
    return u[..., 0::2, :] | (u[..., 1::2, :] << 16)


def _recip(x):
    r = pl.reciprocal(x, approx=True)
    return r * (2.0 - x * r)


def _kernel(x_hbm, k_hbm, v_hbm, sk_hbm, h_hbm, dv_hbm, w_hbm, wo_hbm, gw_hbm,
            f_hbm, g_hbm, z0_hbm, zs_ref, out_hbm,
            k_v, v_v, sk_v, h_v, dv_v, x_v, w_v, wo_v, gw_v, f_v, g_v, z0_v,
            wt_s, wo_s, tmp_s, bq_s, bk_s, bv_s, b_s,
            kf_s, u_s, ht_s, rhs_s, z_s, gg_s, vv_s, y_s, out_s, sems, *tile_refs):
    xp_t, o_t = tile_refs[:NT], tile_refs[NT:2 * NT]
    nsem = [0]

    def dma(src, dst):
        cp = pltpu.make_async_copy(src, dst, sems.at[nsem[0]])
        nsem[0] += 1
        cp.start()
        return cp

    def x_dma(i):
        return dma(x_hbm.at[pl.ds(i * T, T), :], x_v.at[pl.ds(i * T, T), :])

    def a_dma(m):
        rows = pl.ds(m * PC, PC)
        return [dma(k_hbm.at[rows, :], k_v.at[rows, :]),
                dma(v_hbm.at[rows, :], v_v.at[rows, :]),
                dma(h_hbm.at[:, rows], h_v.at[m])]

    cp_w = [dma(w_hbm.at[:, pl.ds(0, D)], w_v.at[0])]
    cp_x = [x_dma(0)]
    cp_z0 = dma(z0_hbm, z0_v)
    cp_w += [dma(w_hbm.at[:, pl.ds(p * D, D)], w_v.at[p]) for p in (1, 2)]
    cp_x.append(x_dma(1))
    cp_small = [dma(sk_hbm, sk_v), dma(dv_hbm, dv_v), dma(gw_hbm, gw_v)]
    cp_a = [a_dma(0)]
    cp_f = dma(f_hbm, f_v)
    cp_wo = dma(wo_hbm, wo_v)
    cp_x += [x_dma(2), x_dma(3)]
    cp_g = dma(g_hbm, g_v)
    cp_a.append(a_dma(1))
    cp_a.append(a_dma(2))
    cp_x += [x_dma(4), x_dma(5)]
    cp_a.append(a_dma(3))
    cp_x += [x_dma(6), x_dma(7)]

    st8 = {"mask": None}

    def link(x, tok):
        if tok is None:
            return x
        if x.shape[0] == 8:
            return jnp.where(st8["mask"], tok, x)
        return jnp.concatenate([jnp.where(st8["mask"], tok, x[0:8]), x[8:]], axis=0)

    def rows(start, size):
        if not CFG["DYN"]:
            return pl.ds(start, size)
        return pl.ds(pl.multiple_of(start + zs_ref[0] * 8, 8), size)

    def slices(res):
        m, n = res.shape
        return [res[r:r + 8, c:c + 128] for c in range(0, n, 128) for r in range(0, m, 8)]

    def proj(i, parts=(0, 1, 2)):
        r0 = i * T
        lo, hi = parts[0] * D, (parts[-1] + 1) * D
        if parts[0] == 0:
            xp_t[i][...] = pltpu.bitcast(x_v[r0:r0 + T, :], U32)
        toks = []
        ns = CFG["NS"]
        for n0 in range(lo, hi, ns):
            n1 = min(n0 + ns, hi)
            res = jax.lax.dot_general(_up(xp_t[i][rows(0, T // 2), :]), _up(wt_s[n0 // 2:n1 // 2, :]),
                                      (((1,), (1,)), ((), ())), preferred_element_type=F32)
            for n in range(n0, n1, 128):
                blk = res[:, n - n0:n - n0 + 128]
                p, c = n // D, (n % D) // 128
                if p == 0:
                    bq_s[c, r0:r0 + T, :] = blk
                elif p == 1:
                    bk_s[c, HALO + r0:HALO + r0 + T, :] = blk
                else:
                    bv_s[c, HALO + r0:HALO + r0 + T, :] = blk
            toks += slices(res)
        return toks

    def outp(i):
        r0 = i * T
        toks = []
        ns = CFG["NS"]
        for n0 in range(0, D, ns):
            n1 = min(n0 + ns, D)
            res = jnp.dot(_up(o_t[i][rows(0, T // 2), :]), _up(wo_s[:, n0:n1]),
                          preferred_element_type=F32)
            for n in range(n0, n1, 128):
                b_s[n // 128, r0:r0 + T, :] = res[:, n - n0:n - n0 + 128]
            toks += slices(res)
        return toks

    def fwd(m):
        toks = []
        ns = CFG["NSF"]
        for s2 in range(4):
            for c in range(NC):
                rhs_s[m, s2, :, c * 128:(c + 1) * 128] = _pk(
                    u_s[c, pl.ds(m * PC + s2, 128, stride=4), :])
                rhs_s[m, s2, :, D + c * 128:D + (c + 1) * 128] = _pk(
                    ht_s[c, pl.ds(m * PC + s2, 128, stride=4), :])
            for n0 in range(0, 2 * D, ns):
                n1 = min(n0 + ns, 2 * D)
                res = jnp.dot(_up(f_v[s2]), _up(rhs_s[m, s2, :, n0:n1]), preferred_element_type=F32)
                z_s[m, s2, :, n0:n1] = res
                toks += slices(res)
        return toks

    def inv(m):
        toks = []
        ns = CFG["NSI"]
        for s2 in range(4):
            for n0 in range(0, D, ns):
                n1 = min(n0 + ns, D)
                res = jnp.dot(_up(g_v[s2]), _up(vv_s[m, s2, :, n0:n1]), preferred_element_type=F32)
                for n in range(n0, n1, 128):
                    y_s[n // 128, pl.ds(m * PC + s2, 128, stride=4), :] = res[:, n - n0:n - n0 + 128]
                toks += slices(res)
        return toks

    def prep_w(p):
        def tr(rc):
            def f(tok):
                for cb in range(NC):
                    blk = w_v[p, rc * 128:(rc + 1) * 128, cb * 128:(cb + 1) * 128].astype(F32)
                    tmp_s[p, rc, cb * 128:(cb + 1) * 128, :] = link(blk, tok).T
                for d in range(DH):
                    r0 = (p * D + d * H) // 2
                    wt_s[r0:r0 + H // 2, rc * 128:(rc + 1) * 128] = _pk(
                        tmp_s[p, rc, pl.ds(d, H, stride=DH), :])
            return f
        return [(250, tr(rc)) for rc in range(NC)]

    def prep_wo(_=None):
        def tr(cc):
            def f(tok):
                tmp_s[3, cc] = link(wo_v[:, cc * 128:(cc + 1) * 128].astype(F32), tok)
                for d in range(DH):
                    wo_s[d * H // 2:(d + 1) * H // 2, cc * 128:(cc + 1) * 128] = _pk(
                        tmp_s[3, cc, pl.ds(d, H, stride=DH), :])
            return f
        return [(160, tr(cc)) for cc in range(NC)]

    def attn_chunk(r, tok):
        ch = 8
        sc = link(jnp.full((ch, 128), QSCALE, F32), tok)
        q = [bq_s[c, r:r + ch, :] * sc for c in range(NC)]
        ls = []
        for w in range(W):
            o = HALO + r - DIL * w
            t = _sum([q[c] * bk_s[c, o:o + ch, :] for c in range(NC)])
            if CFG["ROT3"]:
                t = (t + pltpu.roll(t, 32, 1)) + (pltpu.roll(t, 64, 1) + pltpu.roll(t, 96, 1))
            else:
                t = t + pltpu.roll(t, 64, 1)
                t = t + pltpu.roll(t, 32, 1)
            if r < DIL * w:
                row = jax.lax.broadcasted_iota(jnp.int32, (ch, 128), 0) + r
                t = jnp.where(row >= DIL * w, t, -1e9 * LOG2E)
            ls.append(t)
        m = _tree(ls, jnp.maximum)
        ps = [jnp.exp2(l - m) for l in ls]
        inv_den = _recip(_tree(ps, _add))
        outs = []
        for c in range(NC):
            acc = _sum([ps[w] * bv_s[c, HALO + r - DIL * w:HALO + r - DIL * w + ch, :]
                        for w in range(W)])
            outs.append(acc * inv_den)
        return outs

    def attn(i):
        pend = {}

        def unit(r):
            def f(tok):
                outs = attn_chunk(r, tok)
                if r % 16 == 0:
                    pend[r] = outs
                else:
                    lo = pend.pop(r - 8)
                    for c in range(NC):
                        o_t[i][(r - 8 - i * T) // 2:(r - 8 - i * T) // 2 + 8, c * 128:(c + 1) * 128] = _pk2(lo[c], outs[c])
            return f
        return [(215, unit(r)) for r in range(i * T, (i + 1) * T, 8)]

    def kv_prep(m):
        rb = 64

        def unit(c, r):
            def f(tok):
                cs = slice(c * 128, (c + 1) * 128)
                taps = [link(jnp.broadcast_to(sk_v[j:j + 1, cs].astype(F32), (8, 128)), tok)
                        for j in range(KS)]
                kf_s[c, 8 + r:8 + r + rb, :] = k_v[r:r + rb, cs].astype(F32)
                for rr in range(r, r + rb, 8):
                    ks = kf_s[c, 8 + rr:16 + rr, :] * taps[0]
                    for j in range(1, KS):
                        ks = ks + kf_s[c, 8 + rr - j:16 + rr - j, :] * taps[j]
                    u_s[c, rr:rr + 8, :] = ks * v_v[rr:rr + 8, cs].astype(F32)
            return f
        return [(90, unit(c, r)) for r in range(m * PC, (m + 1) * PC, rb) for c in range(NC)]

    def ht_prep(m):
        def unit(c, j):
            def f(tok):
                blk = h_v[m, c * 128:(c + 1) * 128, j * 128:(j + 1) * 128].astype(F32)
                ht_s[c, m * PC + j * 128:m * PC + (j + 1) * 128, :] = link(blk, tok).T
            return f
        return [(70, unit(c, j)) for c in range(NC) for j in range(PC // 128)]

    def a2_unit(m, c, r, tok):
        ch = 8
        us = slice(c * 128, (c + 1) * 128)
        hs = slice(D + c * 128, D + (c + 1) * 128)

        def ld(mm, ls):
            return [(z_s[mm, k, r:r + ch, ls], z_s[mm, k, 128 + r:128 + r + ch, ls])
                    for k in range(4)]

        zu = ld(m, us)
        zh = ld(m, hs)
        for k in (0, 1):
            zu[k] = (link(zu[k][0], tok), link(zu[k][1], tok))
        for k in ((0, 1) if m == 0 else range(4)):
            zh[k] = (link(zh[k][0], tok), link(zh[k][1], tok))
        if m > 0:
            hp = ld(m - 1, hs)
            if r < 64:
                zh = [(zh[k][0] - hp[k][1], zh[k][1] + hp[k][0]) for k in range(4)]
            else:
                zh = [(zh[k][0] + hp[k][1], zh[k][1] - hp[k][0]) for k in range(4)]
        um = _fft4(zu)
        gm = _fft4(zh)
        if m < NP - 1:
            for k in range(4):
                z_s[m, k, r:r + ch, us] = um[k][0]
                z_s[m, k, 128 + r:128 + r + ch, us] = um[k][1]
                gg_s[m, k, r:r + ch, us] = gm[k][0]
                gg_s[m, k, 128 + r:128 + r + ch, us] = gm[k][1]
        ys = []
        prev = tok
        for k in range(4):
            re = im = None
            for b in range(m, -1, -1):
                a = m - b
                ur, ui = um[k] if b == m else (z_s[b, k, r:r + ch, us],
                                               z_s[b, k, 128 + r:128 + r + ch, us])
                gr, gi = gm[k] if b == 0 else (gg_s[a, k, r:r + ch, us],
                                               gg_s[a, k, 128 + r:128 + r + ch, us])
                if 0 < b < m:
                    ur, ui = link(ur, prev), link(ui, prev)
                pr = ur * gr - ui * gi
                pi = ur * gi + ui * gr
                re = pr if re is None else re + pr
                im = pi if im is None else im + pi
            ys.append((re, im))
            prev = re
        vs = _ifft4(ys)
        for s2 in range(4):
            vv_s[m, s2, r:r + ch, us] = _pk2(vs[s2][0], vs[s2][1])

    def a2(m):
        cost = (92, 128, 168, 208)[m]
        return [(cost, functools.partial(a2_unit, m, c, r))
                for c in range(NC) for r in range(0, 128, 8)]

    out_cps = []

    def final(i):
        def unit(r):
            def f(tok):
                gw = [gw_v[c * 128:(c + 1) * 128].astype(F32).reshape(1, 128) for c in range(NC)]
                dv = [dv_v[c * 128:(c + 1) * 128].astype(F32).reshape(1, 128) for c in range(NC)]
                qf = [link(x_v[r:r + 8, c * 128:(c + 1) * 128].astype(F32), tok) for c in range(NC)]
                z = _tree([qf[c] * gw[c] for c in range(NC)], _add)
                zs = jnp.sum(z, axis=1, keepdims=True)
                g = _recip(1.0 + jnp.exp2(jnp.clip(zs * (-LOG2E), -126.0, 126.0)))
                rb = r - r % 16 + (r % 16) // 8
                for c in range(NC):
                    a = qf[c] * (y_s[c, r:r + 8, :] + u_s[c, r:r + 8, :] * dv[c])
                    b = b_s[c, pl.ds(rb, 8, stride=2), :]
                    out_s[r:r + 8, c * 128:(c + 1) * 128] = (b + g * (a - b)).astype(BF16)
                if r + 8 == (i + 1) * T:
                    out_cps.append(dma(out_s.at[pl.ds(i * T, T), :], out_hbm.at[pl.ds(i * T, T), :]))
            return f
        return [(65, unit(r)) for r in range(i * T, (i + 1) * T, 8)]

    def wait(cps):
        for cp in cps:
            cp.wait()

    mtasks = {"P": proj, "O": outp, "F": fwd, "I": inv,
              "Pq": lambda n: proj(n, (0,)), "Pk": lambda n: proj(n, (1,)), "Pv": lambda n: proj(n, (2,))}
    vtasks = {"AT": attn, "A": a2, "KV": kv_prep, "HT": ht_prep, "FN": final, "PW": prep_w,
              "PWO": prep_wo}
    vcache = {}

    def vunits(spec):
        name, *rng = spec.split(":")
        if name not in vcache:
            base = name.rstrip("0123456789")
            n = int(name[len(base):]) if name[len(base):] else None
            vcache[name] = vtasks[base](n)
        units = vcache[name]
        if rng:
            units = units[int(rng[0]):int(rng[1])]
        return units

    def run(sched):
        for item in sched.split():
            mname, _, vs = item.partition("[")
            toks = None
            if mname != "-":
                base = mname.rstrip("0123456789")
                toks = mtasks[base](int(mname[len(base):]))
            units = []
            for v in vs.rstrip("]").split(","):
                if v:
                    units += vunits(v)
            total = sum(c for c, _ in units)
            acc = 0
            for cost, f in units:
                tok = None
                if toks is not None:
                    frac = CFG["SPAN"] * acc / total
                    tok = toks[min(len(toks) - 1, int(frac * len(toks)))]
                f(tok)
                acc += cost

    def run_plan(plan):
        toks = None
        for mname, units in plan:
            if mname != "-":
                base = mname.rstrip("0123456789")
                toks = mtasks[base](int(mname[len(base):]))
            for vname, j, frac in units:
                tok = None if toks is None else toks[min(len(toks) - 1, int(frac * len(toks)))]
                vunits(vname)[j][1](tok)

    for c in range(NC):
        bk_s[c, 0:HALO, :] = jnp.zeros((HALO, 128), F32)
        bv_s[c, 0:HALO, :] = jnp.zeros((HALO, 128), F32)
        kf_s[c, 0:8, :] = jnp.zeros((8, 128), F32)

    part = CFG["PART"]
    wait([cp_w[0], cp_x[0], cp_z0])
    st8["mask"] = z0_v[...] != 0
    if part in ("all", "first"):
        run("-[PW0]")
        wait([cp_w[1]])
        run("Pq0[PW1]")
        wait([cp_w[2], cp_x[1]])
        run("Pk0[PW2] Pv0[] P1[AT0]")
    else:
        wait(cp_w[1:] + [cp_x[1]])
    wait(cp_small + cp_a[0] + [cp_f, cp_wo, cp_x[2], cp_x[3], cp_g])
    if part in ("all", "first", "r4"):
        run_plan(make_plan(*PLANS[CFG["SCHED"]][0]))
    wait(cp_a[1] + cp_a[2] + cp_a[3] + cp_x[4:8])
    if part in ("all", "second"):
        run_plan(make_plan(*PLANS[CFG["SCHED"]][1]))
    wait(out_cps)
    if part != "all":
        keep = [pltpu.make_async_copy(b, b, sems.at[47]) for b in
                (bq_s, bk_s, bv_s, *o_t, b_s, u_s, ht_s, z_s, gg_s, vv_s, y_s, wo_s, wt_s, kf_s, rhs_s)]
        for cp in keep:
            cp.start()
            cp.wait()


MDUR = {"P": 4800, "O": 1600, "F": 2560, "I": 1280}
VINFO = {"AT": (32, 215, 0, 260), "KV": (40, 90, 0, 40), "HT": (20, 70, 40, 150), "FN": (32, 65, 0, 200),
         "PWO": (5, 160, 0, 60), "A0": (80, 92, 0, 60), "A1": (80, 128, 0, 70), "A2": (80, 168, 0, 80),
         "A3": (80, 208, 0, 90)}


def _vinfo(name):
    base = name if name in VINFO else name.rstrip("0123456789")
    n, cost, gap, lat = VINFO[base]
    if base == "AT":
        gap = CFG["ATGAP"]
    return n, cost, gap, lat


def _vdeps(name):
    base = name.rstrip("0123456789")
    n = int(name[len(base):]) if name[len(base):] else None
    if name == "PWO":
        return [], []
    if base == "AT":
        return ["P%d" % n], []
    if base == "A":
        return ["F%d" % n], (["A%d" % (n - 1)] if n else [])
    if base == "FN":
        return ["O%d" % n, "I%d" % (n // 2)], []
    return [], []


def _mdeps(name):
    base, n = name[0], int(name[1:])
    return {"P": [], "O": ["AT%d" % n] + (["PWO"] if n == 0 else []), "F": ["KV%d" % n, "HT%d" % n],
            "I": ["A%d" % n]}[base]


def make_plan(morder, vprio, done):
    rate = CFG["RATE"]
    morder, vprio, done = morder.split(), vprio.split(), set(done.split())
    mend, mstart, vend = {}, {}, {}
    nxt = {v: 0 for v in vprio}
    last_start = {v: -10**9 for v in vprio}
    starts = []
    mi, mt, vt = 0, 0.0, 0.0
    while mi < len(morder) or any(nxt[v] < _vinfo(v)[0] for v in vprio):
        if mi < len(morder):
            m = morder[mi]
            deps = [d for d in _mdeps(m) if d not in done]
            if all(d in vend for d in deps):
                st = max([mt] + [vend[d] for d in deps])
                mstart[m], mend[m] = st, st + MDUR[m[0]]
                mt = mend[m]
                mi += 1
                continue
        best = None
        for v in vprio:
            n, cost, gap, lat = _vinfo(v)
            if nxt[v] >= n:
                continue
            md, vd = _vdeps(v)
            md = [d for d in md if d not in done]
            vd = [d for d in vd if d not in done]
            if not all(d in mend for d in md) or not all(d in vend for d in vd):
                continue
            st = max([vt, last_start[v] + gap] + [mend[d] for d in md] + [vend[d] for d in vd])
            if best is None or st < best[0] - 1e-9:
                best = (st, v)
        assert best is not None, ("deadlock", morder[mi:], nxt)
        st, v = best
        n, cost, gap, lat = _vinfo(v)
        starts.append((st, v, nxt[v]))
        last_start[v] = st
        nxt[v] += 1
        vt = st + cost / rate
        if nxt[v] == n:
            vend[v] = st + lat
    plan = [(m, []) for m in morder]
    for st, v, j in starts:
        k = max([i for i, m in enumerate(morder) if mstart[m] <= st + 1e-9] or [0])
        m = morder[k]
        frac = min(0.999, max(0.0, (st - mstart[m]) / MDUR[m[0]]))
        plan[k][1].append((v, j, frac))
    if CFG["VERB"]:
        end = max(list(mend.values()) + list(vend.values()))
        print("PLAN end %.0f (M busy %d)" % (end, sum(MDUR[m[0]] for m in morder)))
        for m in morder:
            vs = {}
            for v, j, f in dict(plan)[m]:
                vs.setdefault(v, []).append(j)
            print("  %s %.0f-%.0f %s" % (m, mstart[m], mend[m], " ".join("%s:%d:%d" % (v, js[0], js[-1] + 1) for v, js in vs.items())))
    return plan


PLANS = {
    "A": (("P2 F0 P3 O0 O1 I0 O2 O3", "PWO KV0 HT0 AT1 A0 AT2 AT3 FN0 FN1", "AT0 P0 P1"),
          ("P4 F1 F2 P5 F3 I1 P6 O4 I2 P7 O5 I3 O6 O7",
           "KV1 HT1 KV2 HT2 KV3 HT3 A1 AT4 A2 AT5 A3 AT6 AT7 FN2 FN3 FN4 FN5 FN6 FN7",
           "AT0 AT1 AT2 AT3 O0 O1 O2 O3 I0 A0 PWO P0 P1 P2 P3 F0")),
}


@jax.jit
def pallas_gated_mix__ssm_conv_h3__sliding_local_dilated__prompt_kernel(
    A_q: jax.Array,
    A_k: jax.Array,
    A_v: jax.Array,
    A_shift_k: jax.Array,
    A_ssm_k: jax.Array,
    A_ssm_D: jax.Array,
    B_x: jax.Array,
    B_wqkv: jax.Array,
    B_wo: jax.Array,
    gate_w: jax.Array,
):
    f_np, g_np = _dft_tables()
    f_tab = jnp.asarray(_pack_table(f_np))
    g_tab = jnp.asarray(_pack_table(g_np))
    zeros = jnp.zeros((8, 128), jnp.int32)
    vm = pltpu.VMEM
    scratch = [
        vm((S, D), BF16),
        vm((S, D), BF16),
        vm((KS, D), BF16),
        vm((NP, D, PC), BF16),
        vm((D,), BF16),
        vm((S, D), BF16),
        vm((3, D, D), BF16),
        vm((D, D), BF16),
        vm((D,), BF16),
        vm((4, 128, 128), U32),
        vm((4, 64, 256), U32),
        vm((8, 128), jnp.int32),
        vm((3 * D // 2, D), U32),
        vm((D // 2, D), U32),
        vm((4, NC, D, 128), F32),
        vm((NC, S, 128), F32),
        vm((NC, S + HALO, 128), F32),
        vm((NC, S + HALO, 128), F32),
        vm((NC, S, 128), F32),
        vm((NC, S + 8, 128), F32),
        vm((NC, S, 128), F32),
        vm((NC, S, 128), F32),
        vm((NP, 4, 64, 2 * D), U32),
        vm((NP, 4, 256, 2 * D), F32),
        vm((3, 4, 256, D), F32),
        vm((NP, 4, 128, D), U32),
        vm((NC, S, 128), F32),
        vm((S, D), BF16),
        pltpu.SemaphoreType.DMA((48,)),
    ] + [vm((T // 2, D), U32)] * (2 * NT)
    out = pl.pallas_call(
        _kernel,
        out_shape=jax.ShapeDtypeStruct((S, D), BF16),
        in_specs=[pl.BlockSpec(memory_space=pl.ANY)] * 12 + [pl.BlockSpec(memory_space=pltpu.SMEM)],
        out_specs=pl.BlockSpec(memory_space=pl.ANY),
        scratch_shapes=scratch,
        compiler_params=pltpu.CompilerParams(vmem_limit_bytes=126 * 1024 * 1024),
    )(A_q.reshape(S, D), A_k.reshape(S, D), A_v.reshape(S, D), A_shift_k.T, A_ssm_k, A_ssm_D,
      B_wqkv, B_wo, gate_w, f_tab, g_tab, zeros, jnp.zeros((1,), jnp.int32))
    return out.reshape(1, S, D)
```

```python
import functools

import jax
import jax.numpy as jnp
import numpy as np
import jax.experimental.pallas as pl
import jax.experimental.pallas.tpu as pltpu

S, D = 2048, 640
H, DH, W, DIL = 32, 20, 8, 2
KS = 4
NC = D // 128
T = 256
NT = S // T
HALO = 16
L, PC = 1024, 512
NP = S // PC
LOG2E = 1.4426950408889634
QSCALE = (DH ** -0.5) * LOG2E
F32, BF16, U32 = jnp.float32, jnp.bfloat16, jnp.uint32
import os
CFG = dict(VSTCAP=5.0, START=1, REP=0, STAGE=1, LAG=1500, VCH=0, PROF=0, LAT=2, LA2=1, LKV=2, LHT=3, LFN=3, EARLY=0, FENCE=1, DLD=0, DLHS=0, SPAN=0.92, RATE=2.3, ATGAP=240, VERB=0, DYN=1, NS=128, NSF=128, NSI=128, LA=3, L2=1, LF=2, LK=1, LH=1, GLOBAL=1, ROT3=0, SEQ=1, FULL=1, KCH=1, RHS=1, PART='all', SCHED='G')
for _k in CFG:
    if _k in os.environ:
        CFG[_k] = type(CFG[_k])(os.environ[_k])


def _dft_tables():
    rho = np.arange(128)
    k1 = np.where(rho < 64, 2 * rho, 2 * (rho - 64) + 1)
    s1 = np.arange(128)
    f = np.zeros((4, 256, 128), np.float64)
    for s2 in range(4):
        ph = ((2 * k1[:, None] + 1) * (4 * s1[None, :] + s2)) % (2 * L)
        th = 2 * np.pi * ph / (2 * L)
        f[s2, :128] = np.cos(th)
        f[s2, 128:] = -np.sin(th)
    g = f.transpose(0, 2, 1) * (2.0 / L)
    f = f.reshape(4, 256, 8, 2, 8).transpose(0, 1, 2, 4, 3).reshape(4, 256, 128)
    g = g.reshape(4, 128, 2, 128).transpose(0, 1, 3, 2).reshape(4, 128, 256)
    return f.astype(np.float32), g.astype(np.float32)


def _fft4(z):
    e0 = (z[0][0] + z[2][0], z[0][1] + z[2][1])
    e1 = (z[0][0] - z[2][0], z[0][1] - z[2][1])
    o0 = (z[1][0] + z[3][0], z[1][1] + z[3][1])
    o1 = (z[1][0] - z[3][0], z[1][1] - z[3][1])
    return [
        (e0[0] + o0[0], e0[1] + o0[1]),
        (e1[0] + o1[1], e1[1] - o1[0]),
        (e0[0] - o0[0], e0[1] - o0[1]),
        (e1[0] - o1[1], e1[1] + o1[0]),
    ]


def _ifft4(y):
    a = (y[0][0] + y[2][0], y[0][1] + y[2][1])
    b = (y[0][0] - y[2][0], y[0][1] - y[2][1])
    c = (y[1][0] + y[3][0], y[1][1] + y[3][1])
    d = (y[1][0] - y[3][0], y[1][1] - y[3][1])
    return [
        (a[0] + c[0], a[1] + c[1]),
        (b[0] - d[1], b[1] + d[0]),
        (a[0] - c[0], a[1] - c[1]),
        (b[0] + d[1], b[1] - d[0]),
    ]


def _tree(xs, op):
    xs = list(xs)
    while len(xs) > 1:
        xs = [op(xs[i], xs[i + 1]) if i + 1 < len(xs) else xs[i] for i in range(0, len(xs), 2)]
    return xs[0]


def _add(a, b):
    return a + b


def _sum(xs):
    if CFG['SEQ']:
        return functools.reduce(_add, xs)
    return _tree(xs, _add)


def _pk(x):
    return pltpu.bitcast(x.astype(BF16), U32)


def _pk2(a, b):
    return pltpu.pack_elementwise([a, b], packed_dtype=BF16)


def _up(x):
    return pltpu.bitcast(x, BF16)


def _pack_table(t):
    u = t.astype(jnp.bfloat16).view(np.uint16).astype(np.uint32)
    return u[..., 0::2, :] | (u[..., 1::2, :] << 16)


def _recip(x):
    r = pl.reciprocal(x, approx=True)
    return r * (2.0 - x * r)


def _kernel(x_hbm, k_hbm, v_hbm, sk_hbm, h_hbm, dv_hbm, w_hbm, wo_hbm, gw_hbm,
            f_hbm, g_hbm, z0_hbm, zs_ref, out_hbm,
            k_v, v_v, sk_v, h_v, dv_v, x_v, w_v, wo_v, gw_v, f_v, g_v, z0_v,
            wt_s, wo_s, tmp_s, out_s, sems, *multi):
    multi = list(multi)

    def take(n):
        return [multi.pop(0) for _ in range(n)]
    xp_t, o_t, bq_t, bk_t, bv_t, b_t = (take(NT) for _ in range(6))
    kf_p, u_p, ht_p, rhs_p, z_p, gg_p, vv_p, y_p = (take(NP) for _ in range(8))
    nsem = [0]

    def dma(src, dst):
        cp = pltpu.make_async_copy(src, dst, sems.at[nsem[0]])
        nsem[0] += 1
        cp.start()
        return cp

    def x_dma(i):
        return dma(x_hbm.at[pl.ds(i * T, T), :], x_v.at[pl.ds(i * T, T), :])

    def a_dma(m):
        rows = pl.ds(m * PC, PC)
        return [dma(k_hbm.at[rows, :], k_v.at[rows, :]),
                dma(v_hbm.at[rows, :], v_v.at[rows, :]),
                dma(h_hbm.at[:, rows], h_v.at[m])]

    cp = {}
    cp["z0"] = dma(z0_hbm, z0_v)
    for rc in range(NC):
        cp["wq%d" % rc] = dma(w_hbm.at[pl.ds(rc * 128, 128), pl.ds(0, D)], w_v.at[0, pl.ds(rc * 128, 128), :])
    cp["x0"] = x_dma(0)
    if CFG["START"] == 1:
        cp["x1"] = x_dma(1)
    cp["wk"] = dma(w_hbm.at[:, pl.ds(D, D)], w_v.at[1])
    cp["wv"] = dma(w_hbm.at[:, pl.ds(2 * D, D)], w_v.at[2])
    if CFG["START"] == 0:
        cp["x1"] = x_dma(1)

    def issue_rest():
        cp["a0"] = a_dma(0)
        cp["small"] = [dma(sk_hbm, sk_v), dma(dv_hbm, dv_v), dma(gw_hbm, gw_v)]
        cp["f"] = dma(f_hbm, f_v)
        cp["x2"], cp["x3"] = x_dma(2), x_dma(3)
        cp["g"] = dma(g_hbm, g_v)
        cp["wo"] = dma(wo_hbm, wo_v)
        cp["a1"] = a_dma(1)
        cp["a2"] = a_dma(2)
        cp["x4"], cp["x5"] = x_dma(4), x_dma(5)
        cp["a3"] = a_dma(3)
        cp["x6"], cp["x7"] = x_dma(6), x_dma(7)

    if CFG["STAGE"] == 0:
        issue_rest()

    st8 = {"mask": None, "dirty": {}, "pend": {}, "step": 0}
    zero = zs_ref[0]

    def dyn(i):
        return i + zero if CFG["DLD"] else i

    def link(x, tok):
        if tok is None:
            return x
        if tok.dtype != x.dtype:
            tok = pltpu.bitcast(tok, x.dtype)
        if x.shape == (8, 128):
            return jnp.where(st8["mask"], tok, x)
        head_ = jnp.where(st8["mask"], tok, x[0:8, 0:128])
        if x.shape[1] > 128:
            head_ = jnp.concatenate([head_, x[0:8, 128:]], axis=1)
        return jnp.concatenate([head_, x[8:]], axis=0) if x.shape[0] > 8 else head_

    def wrote(ref, idx):
        st8["dirty"][id(ref)] = (ref, idx)

    def due_step():
        starts = st8["starts"]
        j = st8["step"]
        t = starts[min(j + 1, len(starts) - 1)] + CFG["LAG"]
        while j < len(starts) and starts[j] < t:
            j += 1
        return j

    def end_step():
        if CFG["FENCE"]:
            vals = []
            for ref, idx in st8["dirty"].values():
                idx = (idx[0] + zero,) + tuple(idx[1:])
                vals.append(ref[idx])
            st8["pend"].setdefault(due_step(), []).extend(vals)
        st8["dirty"] = {}
        st8["step"] += 1

    def fenced(w):
        for v in st8["pend"].pop(st8["step"], []):
            w = link(w, v)
        return w

    def slices(res):
        m, n = res.shape
        return [res[r:r + 8, c:c + 128] for r in range(0, m, 8) for c in range(0, n, 128)]

    def proj(i, parts=(0, 1, 2)):
        r0 = i * T

        def dot(n):
            def f():
                if n == 0:
                    xp_t[i][0] = pltpu.bitcast(x_v[r0:r0 + T, :], U32)
                w = fenced(wt_s[n * 64:(n + 1) * 64, :])
                res = jax.lax.dot_general(_up(xp_t[i][zero if CFG['DLHS'] else 0]), _up(w), (((1,), (1,)), ((), ())),
                                          preferred_element_type=F32)
                p, c = divmod(n, NC)
                if p == 0:
                    bq_t[i][c] = res
                    wrote(bq_t[i], (c, slice(0, 8), slice(None)))
                else:
                    dst = bk_t if p == 1 else bv_t
                    dst[i][c, HALO:HALO + T, :] = res
                    wrote(dst[i], (c, slice(HALO, HALO + 8), slice(None)))
                    if i + 1 < NT:
                        dst[i + 1][c, 0:HALO, :] = res[T - HALO:, :]
                return res
            return f
        return [(320, dot(n)) for p in parts for n in range(p * NC, (p + 1) * NC)]

    def outp(i):
        def dot(n):
            def f():
                w = fenced(wo_s[:, n * 128:(n + 1) * 128])
                res = jnp.dot(_up(o_t[i][zero if CFG['DLHS'] else 0]), _up(w), preferred_element_type=F32)
                b_t[i][n] = res
                wrote(b_t[i], (n, slice(0, 8), slice(None)))
                return res
            return f
        return [(320, dot(n)) for n in range(NC)]

    def fwd(m):
        def dot(s2, q):
            def f():
                blocks = FG[q]
                for cb in blocks:
                    src = u_p[m] if cb < NC else ht_p[m]
                    for j in range(8):
                        rhs_p[m][s2, 8 * j:8 * j + 8, cb * 128:(cb + 1) * 128] = _pk2(
                            src[cb % NC, pl.ds(s2 + 64 * j, 8, stride=4), :],
                            src[cb % NC, pl.ds(s2 + 64 * j + 32, 8, stride=4), :])
                lo, hi = blocks[0] * 128, (blocks[-1] + 1) * 128
                w = fenced(rhs_p[m][s2, :, lo:hi])
                res = jnp.dot(_up(f_v[s2]), _up(w), preferred_element_type=F32)
                z_p[m][s2, :, lo:hi] = res
                wrote(z_p[m], (s2, slice(0, 8), slice(lo, lo + 128)))
                return res
            return f
        return [(64 * len(FG[q]), dot(s2, q)) for s2 in range(4) for q in range(len(FG))]

    def inv(m):
        def dot(s2):
            def f():
                w = fenced(vv_p[m][s2])
                res = jnp.dot(_up(g_v[s2]), _up(w), preferred_element_type=F32)
                for c in range(NC):
                    y_p[m][c, pl.ds(s2, 128, stride=4), :] = res[:, c * 128:(c + 1) * 128]
                wrote(y_p[m], (0, pl.ds(s2, 8, stride=4), slice(None)))
                return res
            return f
        return [(320, dot(s2)) for s2 in range(4)]

    def prep_w(p):
        def tr(rc):
            def f(tok):
                for cb in range(NC):
                    blk = w_v[p, rc * 128:(rc + 1) * 128, cb * 128:(cb + 1) * 128].astype(F32)
                    tmp_s[p, rc, cb * 128:(cb + 1) * 128, :] = link(blk, tok).T
                for d in range(DH):
                    r0 = (p * D + d * H) // 2
                    for j in range(2):
                        wt_s[r0 + 8 * j:r0 + 8 * j + 8, rc * 128:(rc + 1) * 128] = _pk2(
                            tmp_s[p, rc, pl.ds(d + 16 * j * DH, 8, stride=DH), :],
                            tmp_s[p, rc, pl.ds(d + (16 * j + 8) * DH, 8, stride=DH), :])
            return f
        return [tr(rc) for rc in range(NC)]

    def prep_wo(_=None):
        def tr(cc):
            def f(tok):
                tmp_s[3, cc] = link(wo_v[:, cc * 128:(cc + 1) * 128].astype(F32), tok)
                for d in range(DH):
                    for j in range(2):
                        r0 = d * H // 2 + 8 * j
                        wo_s[r0:r0 + 8, cc * 128:(cc + 1) * 128] = _pk2(
                            tmp_s[3, cc, pl.ds(d + 16 * j * DH, 8, stride=DH), :],
                            tmp_s[3, cc, pl.ds(d + (16 * j + 8) * DH, 8, stride=DH), :])
            return f
        return [tr(cc) for cc in range(NC)]

    def attn_chunk(i, r, tok):
        ch = 8
        sc = link(jnp.full((ch, 128), QSCALE, F32), tok)
        q = [bq_t[i][dyn(c), r:r + ch, :] * sc for c in range(NC)]
        ls = []
        for w in range(W):
            o = HALO + r - DIL * w
            t = _sum([q[c] * bk_t[i][dyn(c), o:o + ch, :] for c in range(NC)])
            if CFG["ROT3"]:
                t = (t + pltpu.roll(t, 32, 1)) + (pltpu.roll(t, 64, 1) + pltpu.roll(t, 96, 1))
            else:
                t = t + pltpu.roll(t, 64, 1)
                t = t + pltpu.roll(t, 32, 1)
            if i == 0 and r < DIL * w:
                row = jax.lax.broadcasted_iota(jnp.int32, (ch, 128), 0) + r
                t = jnp.where(row >= DIL * w, t, -1e9 * LOG2E)
            ls.append(t)
        m = _tree(ls, jnp.maximum)
        ps = [jnp.exp2(l - m) for l in ls]
        inv_den = _recip(_tree(ps, _add))
        outs = []
        for c in range(NC):
            acc = _sum([ps[w] * bv_t[i][dyn(c), HALO + r - DIL * w:HALO + r - DIL * w + ch, :]
                        for w in range(W)])
            outs.append(acc * inv_den)
        return outs

    def attn(i):
        def unit(r):
            def f(tok):
                lo = attn_chunk(i, r, tok)
                hi = attn_chunk(i, r + 8, tok)
                for c in range(NC):
                    o_t[i][0, r // 2:r // 2 + 8, c * 128:(c + 1) * 128] = _pk2(lo[c], hi[c])
                wrote(o_t[i], (0, slice(r // 2, r // 2 + 8), slice(0, 128)))
                return hi[NC - 1]
            return f
        return [unit(r) for r in range(0, T, 16)]

    def kv_prep(m):
        rb = 64

        def unit(c, r):
            def f(tok):
                cs = slice(c * 128, (c + 1) * 128)
                g0 = m * PC + r
                taps = [link(jnp.broadcast_to(sk_v[j:j + 1, cs].astype(F32), (8, 128)), tok)
                        for j in range(KS)]
                blk = k_v[g0:g0 + rb, cs].astype(F32)
                kf_p[m][c, 8 + r:8 + r + rb, :] = blk
                if r + rb == PC and m + 1 < NP:
                    kf_p[m + 1][c, 0:8, :] = blk[rb - 8:, :]
                for rr in range(r, r + rb, 8):
                    ks = kf_p[m][c, 8 + rr:16 + rr, :] * taps[0]
                    for j in range(1, KS):
                        ks = ks + kf_p[m][c, 8 + rr - j:16 + rr - j, :] * taps[j]
                    uu = ks * v_v[m * PC + rr:m * PC + rr + 8, cs].astype(F32)
                    u_p[m][c, rr:rr + 8, :] = uu
                wrote(u_p[m], (c, slice(r, r + 8), slice(None)))
                return uu
            return f
        return [unit(c, r) for r in range(0, PC, rb) for c in range(NC)]

    def ht_prep(m):
        def unit(c, j):
            def f(tok):
                blk = h_v[m, c * 128:(c + 1) * 128, j * 128:(j + 1) * 128].astype(F32)
                tb = link(blk, tok).T
                if m == 0 and j == 0:
                    row0 = jax.lax.broadcasted_iota(jnp.int32, (8, 128), 0) == 0
                    dvec = dv_v[c * 128:(c + 1) * 128].astype(F32).reshape(1, 128)
                    tb = jnp.concatenate([tb[0:8] + jnp.where(row0, dvec, 0.0), tb[8:]], axis=0)
                ht_p[m][c, j * 128:(j + 1) * 128, :] = tb
                wrote(ht_p[m], (c, slice(j * 128, j * 128 + 8), slice(None)))
                return tb[120:128]
            return f
        return [unit(c, j) for c in range(NC) for j in range(PC // 128)]

    def a2_unit(m, c, r, tok):
        ch = 8
        us = slice(c * 128, (c + 1) * 128)
        hs = slice(D + c * 128, D + (c + 1) * 128)

        def ld(mm, k, ls):
            return (z_p[mm][dyn(k), r:r + ch, ls], z_p[mm][dyn(k), 128 + r:128 + r + ch, ls])

        zu = [ld(m, k, us) for k in range(4)]
        zh = [ld(m, k, hs) for k in range(4)]
        for k in (0, 1):
            zu[k] = (link(zu[k][0], tok), link(zu[k][1], tok))
        for k in ((0, 1) if m == 0 else range(4)):
            zh[k] = (link(zh[k][0], tok), link(zh[k][1], tok))
        if m > 0:
            hp = [ld(m - 1, k, hs) for k in range(4)]
            if r < 64:
                zh = [(zh[k][0] - hp[k][1], zh[k][1] + hp[k][0]) for k in range(4)]
            else:
                zh = [(zh[k][0] + hp[k][1], zh[k][1] - hp[k][0]) for k in range(4)]
        um = _fft4(zu)
        gm = _fft4(zh)
        if m < NP - 1:
            for k in range(4):
                z_p[m][k, r:r + ch, us] = um[k][0]
                z_p[m][k, 128 + r:128 + r + ch, us] = um[k][1]
                gg_p[m][k, r:r + ch, us] = gm[k][0]
                gg_p[m][k, 128 + r:128 + r + ch, us] = gm[k][1]
            wrote(z_p[m], (0, slice(r, r + ch), us))
            wrote(gg_p[m], (0, slice(r, r + ch), us))
        ys = []
        prev = tok
        for k in range(4):
            re = im = None
            for b in range(m, -1, -1):
                a = m - b
                ur, ui = um[k] if b == m else ld(b, k, us)
                gr, gi = gm[k] if b == 0 else (gg_p[a][dyn(k), r:r + ch, us],
                                               gg_p[a][dyn(k), 128 + r:128 + r + ch, us])
                if 0 < b < m:
                    ur, ui = link(ur, prev), link(ui, prev)
                pr = ur * gr - ui * gi
                pi = ur * gi + ui * gr
                re = pr if re is None else re + pr
                im = pi if im is None else im + pi
            ys.append((re, im))
            prev = re
        vs = _ifft4(ys)
        for s2 in range(4):
            vv_p[m][s2, r:r + ch, us] = _pk2(vs[s2][0], vs[s2][1])
        wrote(vv_p[m], (0, slice(r, r + ch), us))
        return vs[3][1]

    def a2(m):
        return [functools.partial(a2_unit, m, c, r) for c in range(NC) for r in range(0, 128, 8)]

    out_cps = []

    def final(i):
        m = i * T // PC

        def unit(r):
            def f(tok):
                g0 = i * T + r
                pr = g0 - m * PC
                gw = [gw_v[c * 128:(c + 1) * 128].astype(F32).reshape(1, 128) for c in range(NC)]
                qf = [link(x_v[g0:g0 + 8, c * 128:(c + 1) * 128].astype(F32), tok) for c in range(NC)]
                z = _tree([qf[c] * gw[c] for c in range(NC)], _add)
                zs = jnp.sum(z, axis=1, keepdims=True)
                g = _recip(1.0 + jnp.exp2(jnp.clip(zs * (-LOG2E), -126.0, 126.0)))
                rb = r - r % 16 + (r % 16) // 8
                for c in range(NC):
                    a = qf[c] * y_p[m][c, pr:pr + 8, :]
                    b = b_t[i][c, pl.ds(rb, 8, stride=2), :]
                    res = b + g * (a - b)
                    out_s[g0:g0 + 8, c * 128:(c + 1) * 128] = res.astype(BF16)
                if CFG["FENCE"]:
                    st8["pend"].setdefault(due_step(), []).append(res)
                piece = T // 4 if i == NT - 1 else T
                if (r + 8) % piece == 0:
                    g1 = g0 + 8 - piece
                    out_cps.append(dma(out_s.at[pl.ds(g1, piece), :], out_hbm.at[pl.ds(g1, piece), :]))
                return res
            return f
        return [unit(r) for r in range(0, T, 8)]

    def wait(names):
        for n in names.split():
            for c_ in (cp[n] if isinstance(cp[n], list) else [cp[n]]):
                c_.wait()
        st8["pend"] = {}
        st8["dirty"] = {}

    mtasks = {"P": proj, "O": outp, "F": fwd, "I": inv,
              "Pq": lambda n: proj(n, (0,)), "Pk": lambda n: proj(n, (1,)), "Pv": lambda n: proj(n, (2,))}
    vtasks = {"AT": attn, "A": a2, "KV": kv_prep, "HT": ht_prep, "FN": final, "PW": prep_w,
              "PWO": prep_wo}
    vcache = {}

    def vunit(name, j):
        if name not in vcache:
            base = name.rstrip("0123456789")
            n = int(name[len(base):]) if name[len(base):] else None
            vcache[name] = vtasks[base](n)
        return vcache[name][j]

    def item_dots(item):
        lists = []
        for part_ in item.split("/"):
            name, *rng = part_.split(":")
            base = name.rstrip("0123456789")
            if name not in mcache:
                mcache[name] = mtasks[base](int(name[len(base):]))
            dots = mcache[name]
            lists.append(dots[int(rng[0]):int(rng[1])] if rng else dots)
        keyed = []
        for dots in lists:
            tot, acc = sum(d for d, _ in dots), 0
            for d, f in dots:
                keyed.append(((acc + 0.5 * d) / tot, d, f))
                acc += d
        keyed.sort(key=lambda x: x[0])
        return [(d, f) for _, d, f in keyed]

    mcache = {}

    def run_plan(plan):
        steps = []
        for mname, units in plan:
            if mname == "-":
                steps.append((0, None, [(v, j, 0.0) for v, j, _ in units]))
                continue
            dots = item_dots(mname)
            total = sum(d for d, _ in dots)
            t0 = 0
            for d, f in dots:
                steps.append((d, f, [(v, j, (fr * total - t0) / d) for v, j, fr in units
                                     if t0 <= fr * total < t0 + d]))
                t0 += d
        starts, t = [], 0
        for d, _, _ in steps:
            starts.append(t)
            t += d
        st8["starts"], st8["step"], st8["pend"], st8["dirty"] = starts + [t], 0, {}, {}
        for d, f, units in steps:
            toks = slices(f()) if f is not None else None
            for v, j, fr in units:
                vunit(v, j)(None if toks is None else toks[int(fr * len(toks))])
            end_step()

    def spread(vname, n):
        return [(vname, j, CFG["SPAN"] * j / n) for j in range(n)]

    for c in range(NC):
        bk_t[0][c, 0:HALO, :] = jnp.zeros((HALO, 128), F32)
        bv_t[0][c, 0:HALO, :] = jnp.zeros((HALO, 128), F32)
        kf_p[0][c, 0:8, :] = jnp.zeros((8, 128), F32)

    part = CFG["PART"]

    def scope(name, fn):
        if CFG["PROF"]:
            with jax.named_scope(name):
                fn()
        else:
            fn()

    scope("w1", lambda: wait("z0 wq0"))
    st8["mask"] = z0_v[...] != 0
    regions = make_plan(*PLANS[CFG["SCHED"]])
    if part in ("all", "first") and CFG["START"] == 1:
        def prep_q():
            for rc in range(NC):
                if rc:
                    wait("wq%d" % rc)
                vunit("PW0", rc)(None)
            wait("x0")
        scope("r1", prep_q)
        scope("r1b", lambda: run_plan([("Pq0", [])]))
        scope("w2", lambda: wait("wk x1"))
        if CFG["STAGE"] == 1:
            issue_rest()
        scope("r2", lambda: run_plan([("Pq1", spread("PW1", NC))]))
        scope("w3", lambda: wait("wv"))
        at0 = spread("AT0", T // 16)
        scope("r3", lambda: run_plan([("Pk0", spread("PW2", NC)), ("Pv0", []),
                                      ("Pk1", [(v, j, 2 * f) for v, j, f in at0[:8]]),
                                      ("Pv1", [(v, j, 2 * f - CFG["SPAN"]) for v, j, f in at0[8:]])]))
    elif part in ("all", "first"):
        scope("r1", lambda: run_plan([("-", spread("PW0", NC))]))
        scope("w2", lambda: wait("wk"))
        if CFG["STAGE"] == 1:
            issue_rest()
        scope("r2", lambda: run_plan([("Pq0", spread("PW1", NC))]))
        scope("w3", lambda: wait("wv x1"))
        scope("r3", lambda: run_plan([("Pk0", spread("PW2", NC)), ("Pv0", []), ("P1", spread("AT0", T // 16))]))
    else:
        wait("wq1 wq2 wq3 wq4 x0 wk")
        if CFG["STAGE"] == 1:
            issue_rest()
        wait("wv x1")
    for k, (wset, plan) in enumerate(regions):
        scope("w%d" % (k + 4), lambda: wait(wset))
        if part in ("all", "first" if k == 0 else "second", "r%d" % (k + 4)):
            if CFG["REP"]:
                def body(_, c_):
                    vcache.clear()
                    mcache.clear()
                    run_plan(plan)
                    return c_
                jax.lax.fori_loop(0, CFG["REP"], body, 0)
            else:
                scope("r%d" % (k + 4), lambda: run_plan(plan))
    scope("wout", lambda: [c_.wait() for c_ in out_cps])
    if part != "all":
        keep = [pltpu.make_async_copy(b, b, sems.at[47]) for b in
                o_t + bq_t + bk_t + bv_t + b_t + kf_p + u_p + ht_p + rhs_p + z_p + gg_p + vv_p + y_p
                + [wo_s, wt_s]]
        for cp in keep:
            cp.start()
            cp.wait()


FG = [(0, 1, 2, 3), (4, 5, 6, 7), (8, 9)]

MDOTS = {"P": [320] * 15, "O": [320] * 5, "F": [256, 256, 128] * 4, "I": [320] * 4}
MST = {"P": 960, "O": 320, "F": 1600, "I": 320}
VINFO = {"AT": (16, 430, 20, 330), "KV": (40, 90, 17, 40), "HT": (20, 70, 16, 150), "FN": (32, 55, 5, 200),
         "PWO": (5, 160, 120, 60), "A0": (80, 92, 20, 60), "A1": (80, 128, 20, 70), "A2": (80, 168, 20, 80),
         "A3": (80, 208, 4, 90)}
WAITS = {"W4": "a0 small f x2 x3 g", "W5": "wo a1 a2 x4 x5 a3 x6 x7"}
BARRIER = 300


def _vinfo(name):
    return VINFO[name if name in VINFO else name.rstrip("0123456789")]


def _vdeps(name):
    base = name.rstrip("0123456789")
    n = int(name[len(base):]) if name[len(base):] else None
    if base == "AT":
        return ["P%d" % n], []
    if base == "A":
        return ["F%d" % n], (["A%d" % (n - 1)] if n else [])
    if base == "FN":
        return ["O%d" % n, "I%d" % (n // 2)], []
    return [], []


def _mdeps(name):
    base, n = name[0], int(name[1:])
    return {"P": [], "O": ["AT%d" % n, "PWO"], "F": ["KV%d" % n, "HT%d" % n], "I": ["A%d" % n]}[base]


def _parts(item):
    out = []
    for p in item.split("/"):
        name, *rng = p.split(":")
        out.append((name, int(rng[0]), int(rng[1])) if rng else (name, 0, len(MDOTS[name[0]])))
    return out


def _idur(item):
    return sum(sum(MDOTS[t[0]][a:b]) for t, a, b in _parts(item))


def _ist(item):
    return sum(MST[t[0]] * sum(MDOTS[t[0]][a:b]) / sum(MDOTS[t[0]]) for t, a, b in _parts(item))


def _avail(name, morder):
    base = name.rstrip("0123456789")
    need = {"KV": "a", "HT": "a", "PWO": "wo"}.get(base)
    if need is None:
        return None
    key = need + name[len(base):]
    for m in morder:
        if m[0] == "W" and key in WAITS[m].split():
            return m
    return None


def make_plan(morder, vprio, done="P0 P1 AT0"):
    rate, vstcap = CFG["RATE"], CFG["VSTCAP"]
    morder, vprio, done = morder.split(), vprio.split(), set(done.split())
    mend, span, vend = {}, {}, {}
    nxt = {v: 0 for v in vprio}
    last_at = [-10**9]
    starts = []
    mi, mt, vt, vbusy = 0, 0.0, 0.0, 0.0

    def m_vst(t):
        for m, (a, b) in span.items():
            if m[0] != "W" and a <= t < b:
                return _ist(m) / (b - a)
        return 0.0

    def unit_time(v, t):
        n, cost, st_, lat = _vinfo(v)
        return max(cost / rate, st_ / max(0.1, vstcap - m_vst(t)))

    def next_unit():
        best = None
        for v in vprio:
            n, cost, st_, lat = _vinfo(v)
            if nxt[v] >= n:
                continue
            md, vd = _vdeps(v)
            w = _avail(v, morder)
            md = [d for d in md + ([w] if w else []) if d not in done]
            vd = [d for d in vd if d not in done]
            if not all(d in mend for d in md) or not all(d in vend for d in vd):
                continue
            gap = CFG["ATGAP"] if v.startswith("AT") else 0
            st = max([vt, last_at[0] + gap if gap else 0] + [mend[d] for d in md] + [vend[d] for d in vd])
            if best is None or st < best[0] - 1e-9:
                best = (st, v)
        return best

    while mi < len(morder) or any(nxt[v] < _vinfo(v)[0] for v in vprio):
        if mi < len(morder):
            m = morder[mi]
            if m[0] == "W":
                cand = next_unit()
                if cand is None or cand[0] + _vinfo(cand[1])[3] >= mt:
                    st = max(mt, vbusy)
                    span[m] = (st, st + (BARRIER if mi else 0))
                    mend[m] = mt = vt = span[m][1]
                    mi += 1
                    continue
            else:
                deps = [d for t, a, b in _parts(m) if a == 0 for d in _mdeps(t) if d not in done]
                if all(d in vend for d in deps):
                    st = max([mt] + [vend[d] for d in deps])
                    span[m] = (st, st + _idur(m))
                    mt = span[m][1]
                    for t, a, b in _parts(m):
                        if b == len(MDOTS[t[0]]):
                            mend[t] = mt
                    mi += 1
                    continue
        best = next_unit()
        assert best is not None, ("deadlock", morder[mi:], nxt)
        st, v = best
        n, cost, st_, lat = _vinfo(v)
        starts.append((st, v, nxt[v]))
        if v.startswith("AT"):
            last_at[0] = st
        nxt[v] += 1
        vt = st + unit_time(v, st)
        vbusy = max(vbusy, st + lat)
        if nxt[v] == n:
            vend[v] = st + lat
    regions, cur, slot = [], None, {}
    for m in morder:
        if m[0] == "W":
            cur = []
            regions.append((WAITS[m], cur))
        else:
            cur.append((m, []))
            slot[m] = cur[-1][1]
    real = [m for m in morder if m[0] != "W"]
    for st, v, j in starts:
        wlast = [m for m in morder if m[0] == "W" and span[m][0] <= st + 1e-9][-1]
        after = [m for m in real if span[m][0] >= span[wlast][1] - 1e-9]
        ok = [m for m in after if span[m][0] <= st + 1e-9]
        m = ok[-1] if ok else after[0]
        slot[m].append((v, j, min(0.999, max(0.0, (st - span[m][0]) / _idur(m)))))
    end = max([b for a, b in span.values()] + list(vend.values()))
    if CFG["VERB"]:
        print("PLAN end %.0f (M busy %d)" % (end, sum(_idur(m) for m in real)))
        for m in morder:
            vs = {}
            for v, j, f in slot.get(m, []):
                vs.setdefault(v, []).append(j)
            print("  %s %.0f-%.0f %s" % (m, span[m][0], span[m][1], " ".join(
                "%s:%d:%d" % (v, js[0], js[-1] + 1) for v, js in vs.items())))
    make_plan.end = end
    return regions


PLANS = {
    "G": ("W4 P2 F0 P3 I0 W5 P4 F1 O0 F2 P5 O1 F3 I1 O2 P6 O3 O4 I2 P7 O5 I3 O6 O7",
          "KV0 HT0 A0 KV1 HT1 PWO KV2 HT2 AT1 KV3 HT3 A1 AT2 AT3 AT4 A2 AT5 A3 AT6 AT7 FN0 FN1 FN2 FN3 FN4 FN5 FN6 FN7"),
    "D": ("W4 P2:0:8 P2:8:15/F0 P3 W5 P4 P5/F1 O0/I0 O1 P6/F2 O2/I1 O3 P7/F3 O4 O5/I2 O6 I3 O7",
          "KV0 HT0 KV1 HT1 PWO A0 AT1 KV2 HT2 AT2 A1 AT3 KV3 HT3 A2 AT4 AT5 AT6 A3 AT7 FN0 FN1 FN2 FN3 FN4 FN5 FN6 FN7"),
    "E": ("W4 P2 F0 P3 W5 P4 I0 O0/F1 P5/F2 O1 I1 P6 O2 O3/F3 O4/I2 P7 O5 O6 I3 O7",
          "KV0 HT0 A0 PWO KV1 HT1 KV2 HT2 AT1 A1 AT2 AT3 KV3 HT3 AT4 A2 AT5 AT6 A3 AT7 FN0 FN1 FN2 FN3 FN4 FN5 FN6 FN7"),
    "F": ("W4 P2:0:8 P2:8:15/F0 P3 W5 P4/I0 P5/F1 O0 P6/F2 O1/I1 O2 O3/F3 P7 O4/I2 O5 O6 I3 O7",
          "KV0 HT0 A0 KV1 HT1 PWO KV2 HT2 AT1 A1 AT2 AT3 KV3 HT3 A2 AT4 AT5 AT6 A3 AT7 FN0 FN1 FN2 FN3 FN4 FN5 FN6 FN7"),
    "B": ("W4 P2 F0 P3 W5 P4 F1 O0 F2 I0 P5 O1 F3 I1 O2 P6 O3 O4 I2 P7 O5 I3 O6 O7",
          "KV0 HT0 KV1 HT1 PWO KV2 HT2 A0 AT1 KV3 HT3 A1 AT2 AT3 AT4 A2 AT5 A3 AT6 AT7 FN0 FN1 FN2 FN3 FN4 FN5 FN6 FN7"),
    "C": ("W4 P2:0:8 P2:8:15/F0 P3 W5 P4 P5/F1 O0/I0 O1 P6/F2 O2 O3 P7/F3 O4/I1 O5 O6/I2 O7:0:1/I3 O7:1:5",
          "KV0 HT0 A0 AT1 KV1 HT1 PWO KV2 HT2 AT2 A1 KV3 HT3 AT3 AT4 A2 AT5 AT6 A3 AT7 FN0 FN1 FN2 FN3 FN4 FN5 FN6 FN7"),
    "T1": ("W4 P2 P3 W5", ""),
}


@jax.jit
def pallas_gated_mix__ssm_conv_h3__sliding_local_dilated__prompt_kernel(
    A_q: jax.Array,
    A_k: jax.Array,
    A_v: jax.Array,
    A_shift_k: jax.Array,
    A_ssm_k: jax.Array,
    A_ssm_D: jax.Array,
    B_x: jax.Array,
    B_wqkv: jax.Array,
    B_wo: jax.Array,
    gate_w: jax.Array,
):
    f_np, g_np = _dft_tables()
    f_tab = jnp.asarray(_pack_table(f_np))
    g_tab = jnp.asarray(_pack_table(g_np))
    zeros = jnp.zeros((8, 128), jnp.int32)
    vm = pltpu.VMEM
    scratch = [
        vm((S, D), BF16),
        vm((S, D), BF16),
        vm((KS, D), BF16),
        vm((NP, D, PC), BF16),
        vm((D,), BF16),
        vm((S, D), BF16),
        vm((3, D, D), BF16),
        vm((D, D), BF16),
        vm((D,), BF16),
        vm((4, 128, 128), U32),
        vm((4, 64, 256), U32),
        vm((8, 128), jnp.int32),
        vm((3 * D // 2, D), U32),
        vm((D // 2, D), U32),
        vm((4, NC, D, 128), F32),
        vm((S, D), BF16),
        pltpu.SemaphoreType.DMA((56,)),
    ]
    scratch += [vm((1, T // 2, D), U32)] * NT
    scratch += [vm((1, T // 2, D), U32)] * NT
    scratch += [vm((NC, T, 128), F32)] * NT
    scratch += [vm((NC, T + HALO, 128), F32)] * NT
    scratch += [vm((NC, T + HALO, 128), F32)] * NT
    scratch += [vm((NC, T, 128), F32)] * NT
    scratch += [vm((NC, PC + 8, 128), F32)] * NP
    scratch += [vm((NC, PC, 128), F32)] * NP
    scratch += [vm((NC, PC, 128), F32)] * NP
    scratch += [vm((4, 64, 2 * D), U32)] * NP
    scratch += [vm((4, 256, 2 * D), F32)] * NP
    scratch += [vm((4, 256, D), F32)] * NP
    scratch += [vm((4, 128, D), U32)] * NP
    scratch += [vm((NC, PC, 128), F32)] * NP
    out = pl.pallas_call(
        _kernel,
        out_shape=jax.ShapeDtypeStruct((S, D), BF16),
        in_specs=[pl.BlockSpec(memory_space=pl.ANY)] * 12 + [pl.BlockSpec(memory_space=pltpu.SMEM)],
        out_specs=pl.BlockSpec(memory_space=pl.ANY),
        scratch_shapes=scratch,
        compiler_params=pltpu.CompilerParams(vmem_limit_bytes=126 * 1024 * 1024),
    )(A_q.reshape(S, D), A_k.reshape(S, D), A_v.reshape(S, D), A_shift_k.T, A_ssm_k, A_ssm_D,
      B_wqkv, B_wo, gate_w, f_tab, g_tab, zeros, jnp.zeros((1,), jnp.int32))
    return out.reshape(1, S, D)
```

```python
import functools

import jax
import jax.numpy as jnp
import numpy as np
import jax.experimental.pallas as pl
import jax.experimental.pallas.tpu as pltpu

S, D = 2048, 640
H, DH, W, DIL = 32, 20, 8, 2
KS = 4
NC = D // 128
T = 256
HALO = 16
L, PC = 1024, 512
NP = S // PC
LOG2E = 1.4426950408889634
QSCALE = (DH ** -0.5) * LOG2E
F32, BF16, U32 = jnp.float32, jnp.bfloat16, jnp.uint32

TSIZES = [256] * 7 + [128] * 2
TSTART = [sum(TSIZES[:i]) for i in range(len(TSIZES))]
NT = len(TSIZES)

RATE = 2.3
RATE_IDLE = 3.0
AT_GAP = 120
LAG_V = 1000
LAG_M = 3000
LAG_FN = 1500
SPAN = 0.92
BARRIER = 300
FG = [(0, 1, 2, 3), (4, 5, 6, 7), (8, 9)]

M_ORDER = ("W4 P2 F0 P3 I0 W5 P4 F1 O0 F2 P5 O1 F3 I1 O2 P6 O3 O4 I2 P7 P8 O5 I3 O6 O7 O8")
V_PRIO = ("KV0 HT0 A0 KV1 HT1 PWO KV2 HT2 AT1 KV3 HT3 A1 AT2 AT3 AT4 A2 AT5 A3 AT6 AT7 AT8 "
          "FN0 FN1 FN2 FN3 FN4 FN5 FN6 FN7 FN8")
WAITS = {"W4": "a0 small f x2 x3 g wo", "W5": "a1 a2 x4 x5 a3 x6 x7"}
MDOTS = {"P": [320] * 15, "O": [320] * 5, "F": [256, 256, 128] * 4, "I": [320] * 4}
VINFO = {"AT": (32, 215, 280), "KV": (40, 90, 40), "HT": (20, 70, 150), "FN": (32, 55, 200),
         "PWO": (5, 160, 60), "A0": (80, 92, 60), "A1": (80, 128, 70), "A2": (80, 168, 80),
         "A3": (80, 208, 90)}


def _dft_tables():
    rho = np.arange(128)
    k1 = np.where(rho < 64, 2 * rho, 2 * (rho - 64) + 1)
    s1 = np.arange(128)
    f = np.zeros((4, 256, 128), np.float64)
    for s2 in range(4):
        ph = ((2 * k1[:, None] + 1) * (4 * s1[None, :] + s2)) % (2 * L)
        th = 2 * np.pi * ph / (2 * L)
        f[s2, :128] = np.cos(th)
        f[s2, 128:] = -np.sin(th)
    g = f.transpose(0, 2, 1) * (2.0 / L)
    f = f.reshape(4, 256, 8, 2, 8).transpose(0, 1, 2, 4, 3).reshape(4, 256, 128)
    g = g.reshape(4, 128, 2, 128).transpose(0, 1, 3, 2).reshape(4, 128, 256)
    return f.astype(np.float32), g.astype(np.float32)


def _pack_table(t):
    u = t.astype(jnp.bfloat16).view(np.uint16).astype(np.uint32)
    return u[..., 0::2, :] | (u[..., 1::2, :] << 16)


def _fft4(z):
    e0 = (z[0][0] + z[2][0], z[0][1] + z[2][1])
    e1 = (z[0][0] - z[2][0], z[0][1] - z[2][1])
    o0 = (z[1][0] + z[3][0], z[1][1] + z[3][1])
    o1 = (z[1][0] - z[3][0], z[1][1] - z[3][1])
    return [
        (e0[0] + o0[0], e0[1] + o0[1]),
        (e1[0] + o1[1], e1[1] - o1[0]),
        (e0[0] - o0[0], e0[1] - o0[1]),
        (e1[0] - o1[1], e1[1] + o1[0]),
    ]


def _ifft4(y):
    a = (y[0][0] + y[2][0], y[0][1] + y[2][1])
    b = (y[0][0] - y[2][0], y[0][1] - y[2][1])
    c = (y[1][0] + y[3][0], y[1][1] + y[3][1])
    d = (y[1][0] - y[3][0], y[1][1] - y[3][1])
    return [
        (a[0] + c[0], a[1] + c[1]),
        (b[0] - d[1], b[1] + d[0]),
        (a[0] - c[0], a[1] - c[1]),
        (b[0] + d[1], b[1] - d[0]),
    ]


def _tree(xs, op):
    xs = list(xs)
    while len(xs) > 1:
        xs = [op(xs[i], xs[i + 1]) if i + 1 < len(xs) else xs[i] for i in range(0, len(xs), 2)]
    return xs[0]


def _add(a, b):
    return a + b


def _sum(xs):
    return functools.reduce(_add, xs)


def _pk2(a, b):
    return pltpu.pack_elementwise([a, b], packed_dtype=BF16)


def _up(x):
    return pltpu.bitcast(x, BF16)


def _recip(x):
    r = pl.reciprocal(x, approx=True)
    return r * (2.0 - x * r)


def _split(name):
    base = name.rstrip("0123456789")
    return base, (int(name[len(base):]) if name[len(base):] else None)


def _vinfo(name):
    base = name if name in VINFO else _split(name)[0]
    n, cost, lat = VINFO[base]
    if base in ("AT", "FN"):
        n = n * TSIZES[_split(name)[1]] // T
    return n, cost, lat


def _mdur(name):
    d = sum(MDOTS[name[0]])
    return d * TSIZES[int(name[1:])] // T if name[0] in "PO" else d


def _vdeps(name):
    base, n = _split(name)
    if base == "AT":
        return ["P%d" % n], []
    if base == "A":
        return ["F%d" % n], (["A%d" % (n - 1)] if n else [])
    if base == "KV" and n:
        return [], ["KV%d" % (n - 1)]
    if base == "FN":
        return ["O%d" % n, "I%d" % (TSTART[n] // PC)], []
    return [], []


def _mdeps(name):
    base, n = name[0], int(name[1:])
    return {"P": [], "O": ["AT%d" % n, "PWO"], "F": ["KV%d" % n, "HT%d" % n], "I": ["A%d" % n]}[base]


def _avail(name, morder):
    base, n = _split(name)
    key = {"KV": "a%s" % n, "HT": "a%s" % n, "PWO": "wo"}.get(base)
    for m in morder:
        if key is not None and m[0] == "W" and key in WAITS[m].split():
            return m
    return None


def _make_plan(morder, vprio, done="P0 P1 AT0"):
    morder, vprio, done = morder.split(), vprio.split(), set(done.split())
    mend, span, vend = {}, {}, {}
    nxt = {v: 0 for v in vprio}
    starts = []
    mi, mt, vt, vbusy, last_at = 0, 0.0, 0.0, 0.0, -1e9

    def next_unit():
        best = None
        for v in vprio:
            if nxt[v] >= _vinfo(v)[0]:
                continue
            md, vd = _vdeps(v)
            w = _avail(v, morder)
            md = [d for d in md + ([w] if w else []) if d not in done]
            vd = [d for d in vd if d not in done]
            if not all(d in mend for d in md) or not all(d in vend for d in vd):
                continue
            st = max([vt, last_at + AT_GAP if v.startswith("AT") else 0]
                     + [mend[d] for d in md] + [vend[d] for d in vd])
            if best is None or st < best[0] - 1e-9:
                best = (st, v)
        return best

    while mi < len(morder) or any(nxt[v] < _vinfo(v)[0] for v in vprio):
        if mi < len(morder):
            m = morder[mi]
            if m[0] == "W":
                cand = next_unit()
                if cand is None or cand[0] + _vinfo(cand[1])[2] >= mt:
                    st = max(mt, vbusy)
                    span[m] = (st, st + (BARRIER if mi else 0))
                    mend[m] = mt = vt = span[m][1]
                    mi += 1
                    continue
            else:
                deps = [d for d in _mdeps(m) if d not in done]
                if all(d in vend for d in deps):
                    st = max([mt] + [vend[d] for d in deps])
                    span[m] = (st, st + _mdur(m))
                    mend[m] = mt = span[m][1]
                    mi += 1
                    continue
        st, v = next_unit()
        n, cost, lat = _vinfo(v)
        starts.append((st, v, nxt[v]))
        if v.startswith("AT"):
            last_at = st
        nxt[v] += 1
        vt = st + cost / (RATE_IDLE if st >= mt else RATE)
        vbusy = max(vbusy, st + lat)
        if nxt[v] == n:
            vend[v] = st + lat
    regions, slot = [], {}
    for m in morder:
        if m[0] == "W":
            regions.append((WAITS[m], []))
        else:
            regions[-1][1].append((m, []))
            slot[m] = regions[-1][1][-1][1]
    real = [m for m in morder if m[0] != "W"]
    for st, v, j in starts:
        wlast = [m for m in morder if m[0] == "W" and span[m][0] <= st + 1e-9][-1]
        after = [m for m in real if span[m][0] >= span[wlast][1] - 1e-9]
        ok = [m for m in after if span[m][0] <= st + 1e-9]
        m = ok[-1] if ok else after[0]
        slot[m].append((v, j, min(0.999, max(0.0, (st - span[m][0]) / _mdur(m)))))
    return regions


def _kernel(x_hbm, k_hbm, v_hbm, sk_hbm, h_hbm, dv_hbm, w_hbm, wo_hbm, gw_hbm,
            f_hbm, g_hbm, z0_hbm, zs_ref, out_hbm,
            k_v, v_v, sk_v, h_v, dv_v, x_v, w_v, wo_v, gw_v, f_v, g_v, z0_v,
            wt_s, wo_s, tmp_s, out_s, sems, *multi):
    multi = list(multi)

    def take(n):
        return [multi.pop(0) for _ in range(n)]
    xp_t, o_t, bq_t, bk_t, bv_t, b_t = (take(NT) for _ in range(6))
    kf_p, u_p, ht_p, rhs_p, z_p, gg_p, vv_p, y_p = (take(NP) for _ in range(8))

    nsem = [0]

    def dma(src, dst):
        cp_ = pltpu.make_async_copy(src, dst, sems.at[nsem[0]])
        nsem[0] += 1
        cp_.start()
        return cp_

    def x_dma(i):
        return [dma(x_hbm.at[pl.ds(i * T, T), :], x_v.at[pl.ds(i * T, T), :])]

    def a_dma(m):
        rows = pl.ds(m * PC, PC)
        return [dma(k_hbm.at[rows, :], k_v.at[rows, :]),
                dma(v_hbm.at[rows, :], v_v.at[rows, :]),
                dma(h_hbm.at[:, rows], h_v.at[m])]

    cp = {"z0": [dma(z0_hbm, z0_v)]}
    for rc in range(NC):
        cp["wq%d" % rc] = [dma(w_hbm.at[pl.ds(rc * 128, 128), pl.ds(0, D)],
                               w_v.at[0, pl.ds(rc * 128, 128), :])]
    cp["x0"] = x_dma(0)
    cp["x1"] = x_dma(1)
    cp["wk"] = [dma(w_hbm.at[:, pl.ds(D, D)], w_v.at[1])]
    cp["wv"] = [dma(w_hbm.at[:, pl.ds(2 * D, D)], w_v.at[2])]

    def issue_rest():
        cp["a0"] = a_dma(0)
        cp["small"] = [dma(sk_hbm, sk_v), dma(dv_hbm, dv_v), dma(gw_hbm, gw_v)]
        cp["f"] = [dma(f_hbm, f_v)]
        cp["x2"], cp["x3"] = x_dma(2), x_dma(3)
        cp["g"] = [dma(g_hbm, g_v)]
        cp["wo"] = [dma(wo_hbm, wo_v)]
        cp["a1"] = a_dma(1)
        cp["a2"] = a_dma(2)
        cp["x4"], cp["x5"] = x_dma(4), x_dma(5)
        cp["a3"] = a_dma(3)
        cp["x6"], cp["x7"] = x_dma(6), x_dma(7)

    st8 = {"mask": None, "dirty": {}, "pend": {}, "step": 0, "starts": [0]}
    zero = zs_ref[0]

    def wait(names):
        for n in names.split():
            for c_ in cp[n]:
                c_.wait()
        st8["pend"], st8["dirty"] = {}, {}

    def link(x, tok):
        if tok is None:
            return x
        if tok.dtype != x.dtype:
            tok = pltpu.bitcast(tok, x.dtype)
        if x.shape == (8, 128):
            return jnp.where(st8["mask"], tok, x)
        head = jnp.where(st8["mask"], tok, x[0:8, 0:128])
        if x.shape[1] > 128:
            head = jnp.concatenate([head, x[0:8, 128:]], axis=1)
        return jnp.concatenate([head, x[8:]], axis=0) if x.shape[0] > 8 else head

    def wrote(ref, lag):
        st8["dirty"][id(ref)] = (ref, lag)

    def due_step(lag):
        starts, j = st8["starts"], st8["step"]
        t = starts[min(j + 1, len(starts) - 1)] + lag
        while j < len(starts) and starts[j] < t:
            j += 1
        return j

    def end_step():
        for ref, lag in st8["dirty"].values():
            lead = jnp.clip(zero, 0, ref.shape[0] - 1)
            st8["pend"].setdefault(due_step(lag), []).append(ref[lead, 0:8, 0:128])
        st8["dirty"] = {}
        st8["step"] += 1

    def fenced(w):
        for v in st8["pend"].pop(st8["step"], []):
            w = link(w, v)
        return w

    def slices(res):
        m, n = res.shape
        return [res[r:r + 8, c:c + 128] for r in range(0, m, 8) for c in range(0, n, 128)]

    def proj(i, parts=(0, 1, 2)):
        r0, tn = TSTART[i], TSIZES[i]

        def dot(n):
            def f():
                if n == 0:
                    xp_t[i][0:tn // 2, :] = pltpu.bitcast(x_v[r0:r0 + tn, :], U32)
                w = fenced(wt_s[n * 64:(n + 1) * 64, :])
                res = jax.lax.dot_general(_up(xp_t[i][0:tn // 2, :]), _up(w),
                                          (((1,), (1,)), ((), ())), preferred_element_type=F32)
                p, c = divmod(n, NC)
                if p == 0:
                    bq_t[i][c, 0:tn, :] = res
                    wrote(bq_t[i], LAG_M)
                else:
                    dst = bk_t if p == 1 else bv_t
                    dst[i][c, HALO:HALO + tn, :] = res
                    wrote(dst[i], LAG_M)
                    if i + 1 < NT:
                        dst[i + 1][c, 0:HALO, :] = res[tn - HALO:, :]
                return res
            return f
        return [(320 * tn // T, dot(n)) for p in parts for n in range(p * NC, (p + 1) * NC)]

    def outp(i):
        tn = TSIZES[i]

        def dot(n):
            def f():
                w = fenced(wo_s[:, n * 128:(n + 1) * 128])
                res = jnp.dot(_up(o_t[i][0, 0:tn // 2, :]), _up(w), preferred_element_type=F32)
                b_t[i][n, 0:tn, :] = res
                wrote(b_t[i], LAG_M)
                return res
            return f
        return [(320 * tn // T, dot(n)) for n in range(NC)]

    def fwd(m):
        def dot(s2, blocks):
            def f():
                for cb in blocks:
                    src = u_p[m] if cb < NC else ht_p[m]
                    for j in range(8):
                        rhs_p[m][s2, 8 * j:8 * j + 8, cb * 128:(cb + 1) * 128] = _pk2(
                            src[cb % NC, pl.ds(s2 + 64 * j, 8, stride=4), :],
                            src[cb % NC, pl.ds(s2 + 64 * j + 32, 8, stride=4), :])
                lo, hi = blocks[0] * 128, (blocks[-1] + 1) * 128
                w = fenced(rhs_p[m][s2, :, lo:hi])
                res = jnp.dot(_up(f_v[s2]), _up(w), preferred_element_type=F32)
                z_p[m][s2, :, lo:hi] = res
                wrote(z_p[m], LAG_M)
                return res
            return f
        return [(64 * len(blocks), dot(s2, blocks)) for s2 in range(4) for blocks in FG]

    def inv(m):
        def dot(s2):
            def f():
                w = fenced(vv_p[m][s2])
                res = jnp.dot(_up(g_v[s2]), _up(w), preferred_element_type=F32)
                for c in range(NC):
                    y_p[m][c, pl.ds(s2, 128, stride=4), :] = res[:, c * 128:(c + 1) * 128]
                wrote(y_p[m], LAG_M)
                return res
            return f
        return [(320, dot(s2)) for s2 in range(4)]

    def head_minor(dst, row0, src, cs):
        for d in range(DH):
            for j in range(2):
                r0 = row0 + d * H // 2 + 8 * j
                dst[r0:r0 + 8, cs] = _pk2(src[pl.ds(d + 16 * j * DH, 8, stride=DH), :],
                                          src[pl.ds(d + (16 * j + 8) * DH, 8, stride=DH), :])

    def prep_w(p):
        def unit(rc):
            def f(tok):
                for cb in range(NC):
                    blk = w_v[p, rc * 128:(rc + 1) * 128, cb * 128:(cb + 1) * 128].astype(F32)
                    tmp_s[p, rc, cb * 128:(cb + 1) * 128, :] = link(blk, tok).T
                head_minor(wt_s, p * D // 2, tmp_s.at[p, rc], slice(rc * 128, (rc + 1) * 128))
            return f
        return [unit(rc) for rc in range(NC)]

    def prep_wo(_):
        def unit(cc):
            def f(tok):
                tmp_s[3, cc] = link(wo_v[:, cc * 128:(cc + 1) * 128].astype(F32), tok)
                head_minor(wo_s, 0, tmp_s.at[3, cc], slice(cc * 128, (cc + 1) * 128))
            return f
        return [unit(cc) for cc in range(NC)]

    def attn(i):
        pend = {}

        def unit(r):
            def f(tok):
                sc = link(jnp.full((8, 128), QSCALE, F32), tok)
                q = [bq_t[i][c, r:r + 8, :] * sc for c in range(NC)]
                ls = []
                for w in range(W):
                    o = HALO + r - DIL * w
                    t = _sum([q[c] * bk_t[i][c, o:o + 8, :] for c in range(NC)])
                    t = (t + pltpu.roll(t, 32, 1)) + (pltpu.roll(t, 64, 1) + pltpu.roll(t, 96, 1))
                    if i == 0 and r < DIL * w:
                        row = jax.lax.broadcasted_iota(jnp.int32, (8, 128), 0) + r
                        t = jnp.where(row >= DIL * w, t, -1e9 * LOG2E)
                    ls.append(t)
                m = _tree(ls, jnp.maximum)
                ps = [jnp.exp2(l - m) for l in ls]
                inv_den = _recip(_tree(ps, _add))
                outs = []
                for c in range(NC):
                    acc = _sum([ps[w] * bv_t[i][c, HALO + r - DIL * w:HALO + r - DIL * w + 8, :]
                                for w in range(W)])
                    outs.append(acc * inv_den)
                if r % 16 == 0:
                    pend[r] = outs
                else:
                    lo, r0 = pend.pop(r - 8), (r - 8) // 2
                    for c in range(NC):
                        o_t[i][0, r0:r0 + 8, c * 128:(c + 1) * 128] = _pk2(lo[c], outs[c])
                    wrote(o_t[i], LAG_V)
            return f
        return [unit(r) for r in range(0, TSIZES[i], 8)]

    def kv_prep(m):
        rb = 64

        def unit(c, r):
            def f(tok):
                cs = slice(c * 128, (c + 1) * 128)
                g0 = m * PC + r
                taps = [link(jnp.broadcast_to(sk_v[j:j + 1, cs].astype(F32), (8, 128)), tok)
                        for j in range(KS)]
                blk = k_v[g0:g0 + rb, cs].astype(F32)
                kf_p[m][c, 8 + r:8 + r + rb, :] = blk
                if r + rb == PC and m + 1 < NP:
                    kf_p[m + 1][c, 0:8, :] = blk[rb - 8:, :]
                for rr in range(r, r + rb, 8):
                    ks = kf_p[m][c, 8 + rr:16 + rr, :] * taps[0]
                    for j in range(1, KS):
                        ks = ks + kf_p[m][c, 8 + rr - j:16 + rr - j, :] * taps[j]
                    u_p[m][c, rr:rr + 8, :] = ks * v_v[m * PC + rr:m * PC + rr + 8, cs].astype(F32)
                wrote(u_p[m], LAG_V)
            return f
        return [unit(c, r) for r in range(0, PC, rb) for c in range(NC)]

    def ht_prep(m):
        def unit(c, j):
            def f(tok):
                blk = h_v[m, c * 128:(c + 1) * 128, j * 128:(j + 1) * 128].astype(F32)
                tb = link(blk, tok).T
                if m == 0 and j == 0:
                    row0 = jax.lax.broadcasted_iota(jnp.int32, (8, 128), 0) == 0
                    dvec = dv_v[c * 128:(c + 1) * 128].astype(F32).reshape(1, 128)
                    tb = jnp.concatenate([tb[0:8] + jnp.where(row0, dvec, 0.0), tb[8:]], axis=0)
                ht_p[m][c, j * 128:(j + 1) * 128, :] = tb
                wrote(ht_p[m], LAG_V)
            return f
        return [unit(c, j) for c in range(NC) for j in range(PC // 128)]

    def spectral_unit(m, c, r, tok):
        us = slice(c * 128, (c + 1) * 128)
        hs = slice(D + c * 128, D + (c + 1) * 128)

        def ld(ref, k, ls):
            return ref[k, r:r + 8, ls], ref[k, 128 + r:128 + r + 8, ls]

        zu = [ld(z_p[m], k, us) for k in range(4)]
        zh = [ld(z_p[m], k, hs) for k in range(4)]
        for k in (0, 1):
            zu[k] = (link(zu[k][0], tok), link(zu[k][1], tok))
        for k in ((0, 1) if m == 0 else range(4)):
            zh[k] = (link(zh[k][0], tok), link(zh[k][1], tok))
        if m > 0:
            hp = [ld(z_p[m - 1], k, hs) for k in range(4)]
            if r < 64:
                zh = [(zh[k][0] - hp[k][1], zh[k][1] + hp[k][0]) for k in range(4)]
            else:
                zh = [(zh[k][0] + hp[k][1], zh[k][1] - hp[k][0]) for k in range(4)]
        um = _fft4(zu)
        gm = _fft4(zh)
        if m < NP - 1:
            for k in range(4):
                z_p[m][k, r:r + 8, us] = um[k][0]
                z_p[m][k, 128 + r:128 + r + 8, us] = um[k][1]
                gg_p[m][k, r:r + 8, us] = gm[k][0]
                gg_p[m][k, 128 + r:128 + r + 8, us] = gm[k][1]
            wrote(z_p[m], LAG_V)
            wrote(gg_p[m], LAG_V)
        ys = []
        prev = tok
        for k in range(4):
            re = im = None
            for b in range(m, -1, -1):
                ur, ui = um[k] if b == m else ld(z_p[b], k, us)
                gr, gi = gm[k] if b == 0 else ld(gg_p[m - b], k, us)
                if 0 < b < m:
                    ur, ui = link(ur, prev), link(ui, prev)
                pr = ur * gr - ui * gi
                pi = ur * gi + ui * gr
                re = pr if re is None else re + pr
                im = pi if im is None else im + pi
            ys.append((re, im))
            prev = re
        vs = _ifft4(ys)
        for s2 in range(4):
            vv_p[m][s2, r:r + 8, us] = _pk2(vs[s2][0], vs[s2][1])
        wrote(vv_p[m], LAG_V)

    def spectral(m):
        return [functools.partial(spectral_unit, m, c, r)
                for c in range(NC) for r in range(0, 128, 8)]

    out_cps = []

    def final(i):
        m = TSTART[i] // PC

        def unit(r):
            def f(tok):
                g0 = TSTART[i] + r
                pr = g0 - m * PC
                gw = [gw_v[c * 128:(c + 1) * 128].astype(F32).reshape(1, 128) for c in range(NC)]
                qf = [link(x_v[g0:g0 + 8, c * 128:(c + 1) * 128].astype(F32), tok)
                      for c in range(NC)]
                z = _tree([qf[c] * gw[c] for c in range(NC)], _add)
                zs = jnp.sum(z, axis=1, keepdims=True)
                g = _recip(1.0 + jnp.exp2(jnp.clip(zs * (-LOG2E), -126.0, 126.0)))
                rb = r - r % 16 + (r % 16) // 8
                for c in range(NC):
                    a = qf[c] * y_p[m][c, pr:pr + 8, :]
                    b = b_t[i][c, pl.ds(rb, 8, stride=2), :]
                    res = b + g * (a - b)
                    out_s[g0:g0 + 8, c * 128:(c + 1) * 128] = res.astype(BF16)
                st8["pend"].setdefault(due_step(LAG_FN), []).append(res)
                piece = TSIZES[i] // 2 if i == NT - 1 else TSIZES[i]
                if (r + 8) % piece == 0:
                    g1 = g0 + 8 - piece
                    out_cps.append(dma(out_s.at[pl.ds(g1, piece), :],
                                       out_hbm.at[pl.ds(g1, piece), :]))
            return f
        return [unit(r) for r in range(0, TSIZES[i], 8)]

    mtasks = {"P": proj, "O": outp, "F": fwd, "I": inv, "Pq": lambda n: proj(n, (0,)),
              "Pk": lambda n: proj(n, (1,)), "Pv": lambda n: proj(n, (2,))}
    vtasks = {"AT": attn, "A": spectral, "KV": kv_prep, "HT": ht_prep, "FN": final,
              "PW": prep_w, "PWO": prep_wo}
    vcache = {}

    def vunit(name, j):
        if name not in vcache:
            base, n = _split(name)
            vcache[name] = vtasks[base](n)
        return vcache[name][j]

    def run_plan(plan):
        steps = []
        for mname, units in plan:
            base, n = _split(mname)
            dots = mtasks[base](n)
            total, t0 = sum(d for d, _ in dots), 0
            for d, f in dots:
                steps.append((d, f, [(v, j, (fr * total - t0) / d) for v, j, fr in units
                                     if t0 <= fr * total < t0 + d]))
                t0 += d
        starts, t = [], 0
        for d, _, _ in steps:
            starts.append(t)
            t += d
        st8["starts"], st8["step"], st8["pend"], st8["dirty"] = starts + [t], 0, {}, {}
        for d, f, units in steps:
            toks = slices(f())
            for v, j, fr in units:
                vunit(v, j)(toks[int(fr * len(toks))])
            end_step()

    def spread(vname, lo, hi):
        return [(vname, j, SPAN * (j - lo) / (hi - lo)) for j in range(lo, hi)]

    for ref in o_t + bq_t + bk_t + bv_t + b_t + u_p + ht_p + y_p + z_p + gg_p + vv_p:
        for k in range(ref.shape[0]):
            ref[k, 0:8, 0:128] = jnp.zeros((8, 128), ref.dtype)
    for c in range(NC):
        bk_t[0][c, 0:HALO, :] = jnp.zeros((HALO, 128), F32)
        bv_t[0][c, 0:HALO, :] = jnp.zeros((HALO, 128), F32)
        kf_p[0][c, 0:8, :] = jnp.zeros((8, 128), F32)

    wait("z0 wq0")
    st8["mask"] = z0_v[...] != 0
    for rc in range(NC):
        if rc:
            wait("wq%d" % rc)
        vunit("PW0", rc)(None)
    wait("x0")
    run_plan([("Pq0", [])])
    wait("wk x1")
    issue_rest()
    run_plan([("Pq1", spread("PW1", 0, NC))])
    wait("wv")
    run_plan([("Pk0", spread("PW2", 0, NC)), ("Pv0", []),
              ("Pk1", spread("AT0", 0, 16)), ("Pv1", spread("AT0", 16, 32))])
    for wset, plan in _make_plan(M_ORDER, V_PRIO):
        wait(wset)
        run_plan(plan)
    for c_ in out_cps:
        c_.wait()


@jax.jit
def pallas_gated_mix__ssm_conv_h3__sliding_local_dilated__prompt_kernel(
    A_q: jax.Array,
    A_k: jax.Array,
    A_v: jax.Array,
    A_shift_k: jax.Array,
    A_ssm_k: jax.Array,
    A_ssm_D: jax.Array,
    B_x: jax.Array,
    B_wqkv: jax.Array,
    B_wo: jax.Array,
    gate_w: jax.Array,
):
    f_np, g_np = _dft_tables()
    vm = pltpu.VMEM
    scratch = [
        vm((S, D), BF16),
        vm((S, D), BF16),
        vm((KS, D), BF16),
        vm((NP, D, PC), BF16),
        vm((D,), BF16),
        vm((S, D), BF16),
        vm((3, D, D), BF16),
        vm((D, D), BF16),
        vm((D,), BF16),
        vm((4, 128, 128), U32),
        vm((4, 64, 256), U32),
        vm((8, 128), jnp.int32),
        vm((3 * D // 2, D), U32),
        vm((D // 2, D), U32),
        vm((4, NC, D, 128), F32),
        vm((S, D), BF16),
        pltpu.SemaphoreType.DMA((48,)),
    ]
    scratch += [vm((T // 2, D), U32)] * NT
    scratch += [vm((2, T // 2, D), U32)] * NT
    scratch += [vm((NC, T, 128), F32)] * NT
    scratch += [vm((NC, T + HALO, 128), F32)] * NT
    scratch += [vm((NC, T + HALO, 128), F32)] * NT
    scratch += [vm((NC, T, 128), F32)] * NT
    scratch += [vm((NC, PC + 8, 128), F32)] * NP
    scratch += [vm((NC, PC, 128), F32)] * NP
    scratch += [vm((NC, PC, 128), F32)] * NP
    scratch += [vm((4, 64, 2 * D), U32)] * NP
    scratch += [vm((4, 256, 2 * D), F32)] * NP
    scratch += [vm((4, 256, D), F32)] * NP
    scratch += [vm((4, 128, D), U32)] * NP
    scratch += [vm((NC, PC, 128), F32)] * NP
    out = pl.pallas_call(
        _kernel,
        out_shape=jax.ShapeDtypeStruct((S, D), BF16),
        in_specs=[pl.BlockSpec(memory_space=pl.ANY)] * 12
        + [pl.BlockSpec(memory_space=pltpu.SMEM)],
        out_specs=pl.BlockSpec(memory_space=pl.ANY),
        scratch_shapes=scratch,
        compiler_params=pltpu.CompilerParams(vmem_limit_bytes=126 * 1024 * 1024),
    )(A_q.reshape(S, D), A_k.reshape(S, D), A_v.reshape(S, D), A_shift_k.T, A_ssm_k, A_ssm_D,
      B_wqkv, B_wo, gate_w, jnp.asarray(_pack_table(f_np)), jnp.asarray(_pack_table(g_np)),
      jnp.asarray(np.zeros((8, 128), np.int32)), jnp.asarray(np.zeros((1,), np.int32)))
    return out.reshape(1, S, D)
```

```python
import functools

import jax
import jax.numpy as jnp
import numpy as np
import jax.experimental.pallas as pl
import jax.experimental.pallas.tpu as pltpu

S, D = 2048, 640
H, DH, W, DIL = 32, 20, 8, 2
KS = 4
NC = D // 128
T = 256
HALO = 16
L, PC = 1024, 512
NP = S // PC
LOG2E = 1.4426950408889634
QSCALE = (DH ** -0.5) * LOG2E
F32, BF16, U32 = jnp.float32, jnp.bfloat16, jnp.uint32

TSIZES = [256] * 7 + [128] * 2
TSTART = [sum(TSIZES[:i]) for i in range(len(TSIZES))]
NT = len(TSIZES)

RATE = 2.3
RATE_IDLE = 3.0
AT_GAP = 120
LAG_V = 1000
LAG_M = 3000
LAG_FN = 1500
SPAN = 0.92
BARRIER = 300
FG = [(0, 1, 2, 3), (4, 5, 6, 7), (8, 9)]

M_ORDER = ("W4 P2 F0 P3 I0 W5 P4 F1 O0 F2 P5 O1 F3 I1 O2 P6 O3 O4 I2 P7 P8 O5 I3 O6 O7 O8")
V_PRIO = ("KV0 HT0 A0 KV1 HT1 PWO KV2 HT2 AT1 KV3 HT3 A1 AT2 AT3 AT4 A2 AT5 A3 AT6 AT7 AT8 "
          "FN0 FN1 FN2 FN3 FN4 FN5 FN6 FN7 FN8")
WAITS = {"W4": "a0 small f x2 x3 g wo", "W5": "a1 a2 x4 x5 a3 x6 x7"}
MDOTS = {"P": [320] * 15, "O": [320] * 5, "F": [256, 256, 128] * 4, "I": [320] * 4}
VINFO = {"AT": (32, 215, 280), "KV": (40, 86, 40), "HT": (20, 70, 150), "FN": (32, 52, 200),
         "PWO": (5, 160, 60), "A0": (80, 92, 60), "A1": (80, 128, 70), "A2": (80, 168, 80),
         "A3": (80, 208, 90)}


def _dft_tables():
    rho = np.arange(128)
    k1 = np.where(rho < 64, 2 * rho, 2 * (rho - 64) + 1)
    s1 = np.arange(128)
    f = np.zeros((4, 256, 128), np.float64)
    for s2 in range(4):
        ph = ((2 * k1[:, None] + 1) * (4 * s1[None, :] + s2)) % (2 * L)
        th = 2 * np.pi * ph / (2 * L)
        f[s2, :128] = np.cos(th)
        f[s2, 128:] = -np.sin(th)
    g = f.transpose(0, 2, 1) * (2.0 / L)
    f = f.reshape(4, 256, 8, 2, 8).transpose(0, 1, 2, 4, 3).reshape(4, 256, 128)
    g = g.reshape(4, 128, 2, 128).transpose(0, 1, 3, 2).reshape(4, 128, 256)
    return f.astype(np.float32), g.astype(np.float32)


def _pack_table(t):
    u = t.astype(jnp.bfloat16).view(np.uint16).astype(np.uint32)
    return u[..., 0::2, :] | (u[..., 1::2, :] << 16)


def _fft4(z):
    e0 = (z[0][0] + z[2][0], z[0][1] + z[2][1])
    e1 = (z[0][0] - z[2][0], z[0][1] - z[2][1])
    o0 = (z[1][0] + z[3][0], z[1][1] + z[3][1])
    o1 = (z[1][0] - z[3][0], z[1][1] - z[3][1])
    return [
        (e0[0] + o0[0], e0[1] + o0[1]),
        (e1[0] + o1[1], e1[1] - o1[0]),
        (e0[0] - o0[0], e0[1] - o0[1]),
        (e1[0] - o1[1], e1[1] + o1[0]),
    ]


def _ifft4(y):
    a = (y[0][0] + y[2][0], y[0][1] + y[2][1])
    b = (y[0][0] - y[2][0], y[0][1] - y[2][1])
    c = (y[1][0] + y[3][0], y[1][1] + y[3][1])
    d = (y[1][0] - y[3][0], y[1][1] - y[3][1])
    return [
        (a[0] + c[0], a[1] + c[1]),
        (b[0] - d[1], b[1] + d[0]),
        (a[0] - c[0], a[1] - c[1]),
        (b[0] + d[1], b[1] - d[0]),
    ]


def _tree(xs, op):
    xs = list(xs)
    while len(xs) > 1:
        xs = [op(xs[i], xs[i + 1]) if i + 1 < len(xs) else xs[i] for i in range(0, len(xs), 2)]
    return xs[0]


def _add(a, b):
    return a + b


def _sum(xs):
    return functools.reduce(_add, xs)


def _pk2(a, b):
    return pltpu.pack_elementwise([a, b], packed_dtype=BF16)


def _up(x):
    return pltpu.bitcast(x, BF16)


def _recip(x):
    r = pl.reciprocal(x, approx=True)
    return r * (2.0 - x * r)


def _split(name):
    base = name.rstrip("0123456789")
    return base, (int(name[len(base):]) if name[len(base):] else None)


def _vinfo(name):
    base = name if name in VINFO else _split(name)[0]
    n, cost, lat = VINFO[base]
    if base in ("AT", "FN"):
        n = n * TSIZES[_split(name)[1]] // T
    return n, cost, lat


def _mdur(name):
    d = sum(MDOTS[name[0]])
    return d * TSIZES[int(name[1:])] // T if name[0] in "PO" else d


def _vdeps(name):
    base, n = _split(name)
    if base == "AT":
        return ["P%d" % n], []
    if base == "A":
        return ["F%d" % n], (["A%d" % (n - 1)] if n else [])
    if base == "KV" and n:
        return [], ["KV%d" % (n - 1)]
    if base == "FN":
        return ["O%d" % n, "I%d" % (TSTART[n] // PC)], []
    return [], []


def _mdeps(name):
    base, n = name[0], int(name[1:])
    return {"P": [], "O": ["AT%d" % n, "PWO"], "F": ["KV%d" % n, "HT%d" % n], "I": ["A%d" % n]}[base]


def _avail(name, morder):
    base, n = _split(name)
    key = {"KV": "a%s" % n, "HT": "a%s" % n, "PWO": "wo"}.get(base)
    for m in morder:
        if key is not None and m[0] == "W" and key in WAITS[m].split():
            return m
    return None


def _make_plan(morder, vprio, done="P0 P1 AT0"):
    morder, vprio, done = morder.split(), vprio.split(), set(done.split())
    mend, span, vend = {}, {}, {}
    nxt = {v: 0 for v in vprio}
    starts = []
    mi, mt, vt, vbusy, last_at = 0, 0.0, 0.0, 0.0, -1e9

    def next_unit():
        best = None
        for v in vprio:
            if nxt[v] >= _vinfo(v)[0]:
                continue
            md, vd = _vdeps(v)
            w = _avail(v, morder)
            md = [d for d in md + ([w] if w else []) if d not in done]
            vd = [d for d in vd if d not in done]
            if not all(d in mend for d in md) or not all(d in vend for d in vd):
                continue
            st = max([vt, last_at + AT_GAP if v.startswith("AT") else 0]
                     + [mend[d] for d in md] + [vend[d] for d in vd])
            if best is None or st < best[0] - 1e-9:
                best = (st, v)
        return best

    while mi < len(morder) or any(nxt[v] < _vinfo(v)[0] for v in vprio):
        if mi < len(morder):
            m = morder[mi]
            if m[0] == "W":
                cand = next_unit()
                if cand is None or cand[0] + _vinfo(cand[1])[2] >= mt:
                    st = max(mt, vbusy)
                    span[m] = (st, st + (BARRIER if mi else 0))
                    mend[m] = mt = vt = span[m][1]
                    mi += 1
                    continue
            else:
                deps = [d for d in _mdeps(m) if d not in done]
                if all(d in vend for d in deps):
                    st = max([mt] + [vend[d] for d in deps])
                    span[m] = (st, st + _mdur(m))
                    mend[m] = mt = span[m][1]
                    mi += 1
                    continue
        st, v = next_unit()
        n, cost, lat = _vinfo(v)
        starts.append((st, v, nxt[v]))
        if v.startswith("AT"):
            last_at = st
        nxt[v] += 1
        vt = st + cost / (RATE_IDLE if st >= mt else RATE)
        vbusy = max(vbusy, st + lat)
        if nxt[v] == n:
            vend[v] = st + lat
    regions, slot = [], {}
    for m in morder:
        if m[0] == "W":
            regions.append((WAITS[m], []))
        else:
            regions[-1][1].append((m, []))
            slot[m] = regions[-1][1][-1][1]
    real = [m for m in morder if m[0] != "W"]
    for st, v, j in starts:
        wlast = [m for m in morder if m[0] == "W" and span[m][0] <= st + 1e-9][-1]
        after = [m for m in real if span[m][0] >= span[wlast][1] - 1e-9]
        ok = [m for m in after if span[m][0] <= st + 1e-9]
        m = ok[-1] if ok else after[0]
        slot[m].append((v, j, min(0.999, max(0.0, (st - span[m][0]) / _mdur(m)))))
    return regions


def _kernel(x_hbm, k_hbm, v_hbm, sk_hbm, h_hbm, dv_hbm, w_hbm, wo_hbm, gw_hbm,
            f_hbm, g_hbm, z0_hbm, zs_ref, out_hbm,
            k_v, v_v, sk_v, h_v, dv_v, x_v, w_v, wo_v, gw_v, f_v, g_v, z0_v,
            wt_s, wo_s, tmp_s, bc_s, out_s, sems, *multi):
    multi = list(multi)

    def take(n):
        return [multi.pop(0) for _ in range(n)]
    xp_t, o_t, bq_t, bk_t, bv_t, b_t = (take(NT) for _ in range(6))
    kf_p, u_p, ht_p, rhs_p, z_p, gg_p, vv_p, y_p = (take(NP) for _ in range(8))

    nsem = [0]

    def dma(src, dst):
        cp_ = pltpu.make_async_copy(src, dst, sems.at[nsem[0]])
        nsem[0] += 1
        cp_.start()
        return cp_

    def x_dma(i):
        return [dma(x_hbm.at[pl.ds(i * T, T), :], x_v.at[pl.ds(i * T, T), :])]

    def a_dma(m):
        rows = pl.ds(m * PC, PC)
        return [dma(k_hbm.at[rows, :], k_v.at[rows, :]),
                dma(v_hbm.at[rows, :], v_v.at[rows, :]),
                dma(h_hbm.at[:, rows], h_v.at[m])]

    cp = {"z0": [dma(z0_hbm, z0_v)]}
    for rc in range(NC):
        cp["wq%d" % rc] = [dma(w_hbm.at[pl.ds(rc * 128, 128), pl.ds(0, D)],
                               w_v.at[0, pl.ds(rc * 128, 128), :])]
    cp["x0"] = x_dma(0)
    cp["x1"] = x_dma(1)
    cp["wk"] = [dma(w_hbm.at[:, pl.ds(D, D)], w_v.at[1])]
    cp["wv"] = [dma(w_hbm.at[:, pl.ds(2 * D, D)], w_v.at[2])]

    def issue_rest():
        cp["a0"] = a_dma(0)
        cp["small"] = [dma(sk_hbm, sk_v), dma(dv_hbm, dv_v), dma(gw_hbm, gw_v)]
        cp["f"] = [dma(f_hbm, f_v)]
        cp["x2"], cp["x3"] = x_dma(2), x_dma(3)
        cp["g"] = [dma(g_hbm, g_v)]
        cp["wo"] = [dma(wo_hbm, wo_v)]
        cp["a1"] = a_dma(1)
        cp["a2"] = a_dma(2)
        cp["x4"], cp["x5"] = x_dma(4), x_dma(5)
        cp["a3"] = a_dma(3)
        cp["x6"], cp["x7"] = x_dma(6), x_dma(7)

    st8 = {"mask": None, "dirty": {}, "pend": {}, "step": 0, "starts": [0]}
    zero = zs_ref[0]

    def wait(names):
        for n in names.split():
            for c_ in cp[n]:
                c_.wait()
        st8["pend"], st8["dirty"] = {}, {}

    def link(x, tok):
        if tok is None:
            return x
        if tok.dtype != x.dtype:
            tok = pltpu.bitcast(tok, x.dtype)
        if x.shape == (8, 128):
            return jnp.where(st8["mask"], tok, x)
        head = jnp.where(st8["mask"], tok, x[0:8, 0:128])
        if x.shape[1] > 128:
            head = jnp.concatenate([head, x[0:8, 128:]], axis=1)
        return jnp.concatenate([head, x[8:]], axis=0) if x.shape[0] > 8 else head

    def wrote(ref, lag):
        st8["dirty"][id(ref)] = (ref, lag)

    def due_step(lag):
        starts, j = st8["starts"], st8["step"]
        t = starts[min(j + 1, len(starts) - 1)] + lag
        while j < len(starts) and starts[j] < t:
            j += 1
        return j

    def end_step():
        for ref, lag in st8["dirty"].values():
            lead = jnp.clip(zero, 0, ref.shape[0] - 1)
            st8["pend"].setdefault(due_step(lag), []).append(ref[lead, 0:8, 0:128])
        st8["dirty"] = {}
        st8["step"] += 1

    def fenced(w):
        for v in st8["pend"].pop(st8["step"], []):
            w = link(w, v)
        return w

    def slices(res):
        m, n = res.shape
        return [res[r:r + 8, c:c + 128] for r in range(0, m, 8) for c in range(0, n, 128)]

    def proj(i, parts=(0, 1, 2)):
        r0, tn = TSTART[i], TSIZES[i]

        def dot(n):
            def f():
                if n == 0:
                    xp_t[i][0:tn // 2, :] = pltpu.bitcast(x_v[r0:r0 + tn, :], U32)
                w = fenced(wt_s[n * 64:(n + 1) * 64, :])
                res = jax.lax.dot_general(_up(xp_t[i][0:tn // 2, :]), _up(w),
                                          (((1,), (1,)), ((), ())), preferred_element_type=F32)
                p, c = divmod(n, NC)
                if p == 0:
                    bq_t[i][c, 0:tn, :] = res
                    wrote(bq_t[i], LAG_M)
                else:
                    dst = bk_t if p == 1 else bv_t
                    dst[i][c, HALO:HALO + tn, :] = res
                    wrote(dst[i], LAG_M)
                    if i + 1 < NT:
                        dst[i + 1][c, 0:HALO, :] = res[tn - HALO:, :]
                return res
            return f
        return [(320 * tn // T, dot(n)) for p in parts for n in range(p * NC, (p + 1) * NC)]

    def outp(i):
        tn = TSIZES[i]

        def dot(n):
            def f():
                w = fenced(wo_s[:, n * 128:(n + 1) * 128])
                res = jnp.dot(_up(o_t[i][0, 0:tn // 2, :]), _up(w), preferred_element_type=F32)
                b_t[i][n, 0:tn, :] = res
                wrote(b_t[i], LAG_M)
                return res
            return f
        return [(320 * tn // T, dot(n)) for n in range(NC)]

    def fwd(m):
        def dot(s2, blocks):
            def f():
                for cb in blocks:
                    src = u_p[m] if cb < NC else ht_p[m]
                    for j in range(8):
                        rhs_p[m][s2, 8 * j:8 * j + 8, cb * 128:(cb + 1) * 128] = _pk2(
                            src[cb % NC, pl.ds(s2 + 64 * j, 8, stride=4), :],
                            src[cb % NC, pl.ds(s2 + 64 * j + 32, 8, stride=4), :])
                lo, hi = blocks[0] * 128, (blocks[-1] + 1) * 128
                w = fenced(rhs_p[m][s2, :, lo:hi])
                res = jnp.dot(_up(f_v[s2]), _up(w), preferred_element_type=F32)
                z_p[m][s2, :, lo:hi] = res
                wrote(z_p[m], LAG_M)
                return res
            return f
        return [(64 * len(blocks), dot(s2, blocks)) for s2 in range(4) for blocks in FG]

    def inv(m):
        def dot(s2):
            def f():
                w = fenced(vv_p[m][s2])
                res = jnp.dot(_up(g_v[s2]), _up(w), preferred_element_type=F32)
                for c in range(NC):
                    y_p[m][c, pl.ds(s2, 128, stride=4), :] = res[:, c * 128:(c + 1) * 128]
                wrote(y_p[m], LAG_M)
                return res
            return f
        return [(320, dot(s2)) for s2 in range(4)]

    def head_minor(dst, row0, src, cs):
        for d in range(DH):
            for j in range(2):
                r0 = row0 + d * H // 2 + 8 * j
                dst[r0:r0 + 8, cs] = _pk2(src[pl.ds(d + 16 * j * DH, 8, stride=DH), :],
                                          src[pl.ds(d + (16 * j + 8) * DH, 8, stride=DH), :])

    def prep_w(p):
        def unit(rc):
            def f(tok):
                for cb in range(NC):
                    blk = w_v[p, rc * 128:(rc + 1) * 128, cb * 128:(cb + 1) * 128].astype(F32)
                    tmp_s[p, rc, cb * 128:(cb + 1) * 128, :] = link(blk, tok).T
                head_minor(wt_s, p * D // 2, tmp_s.at[p, rc], slice(rc * 128, (rc + 1) * 128))
            return f
        return [unit(rc) for rc in range(NC)]

    def prep_wo(_):
        def unit(cc):
            def f(tok):
                tmp_s[3, cc] = link(wo_v[:, cc * 128:(cc + 1) * 128].astype(F32), tok)
                head_minor(wo_s, 0, tmp_s.at[3, cc], slice(cc * 128, (cc + 1) * 128))
            return f
        return [unit(cc) for cc in range(NC)]

    def attn(i):
        pend = {}

        def unit(r):
            def f(tok):
                sc = link(jnp.full((8, 128), QSCALE, F32), tok)
                q = [bq_t[i][c, r:r + 8, :] * sc for c in range(NC)]
                ls = []
                for w in range(W):
                    o = HALO + r - DIL * w
                    t = _sum([q[c] * bk_t[i][c, o:o + 8, :] for c in range(NC)])
                    t = (t + pltpu.roll(t, 32, 1)) + (pltpu.roll(t, 64, 1) + pltpu.roll(t, 96, 1))
                    if i == 0 and r < DIL * w:
                        row = jax.lax.broadcasted_iota(jnp.int32, (8, 128), 0) + r
                        t = jnp.where(row >= DIL * w, t, -1e9 * LOG2E)
                    ls.append(t)
                m = _tree(ls, jnp.maximum)
                ps = [jnp.exp2(l - m) for l in ls]
                inv_den = _recip(_tree(ps, _add))
                outs = []
                for c in range(NC):
                    acc = _sum([ps[w] * bv_t[i][c, HALO + r - DIL * w:HALO + r - DIL * w + 8, :]
                                for w in range(W)])
                    outs.append(acc * inv_den)
                if r % 16 == 0:
                    pend[r] = outs
                else:
                    lo, r0 = pend.pop(r - 8), (r - 8) // 2
                    for c in range(NC):
                        o_t[i][0, r0:r0 + 8, c * 128:(c + 1) * 128] = _pk2(lo[c], outs[c])
                    wrote(o_t[i], LAG_V)
            return f
        return [unit(r) for r in range(0, TSIZES[i], 8)]

    def kv_prep(m):
        rb = 64

        def unit(c, r):
            def f(tok):
                cs = slice(c * 128, (c + 1) * 128)
                g0 = m * PC + r
                taps = [link(bc_s[(1 + j) * NC + c], tok) for j in range(KS)]
                blk = k_v[g0:g0 + rb, cs].astype(F32)
                kf_p[m][c, 8 + r:8 + r + rb, :] = blk
                if r + rb == PC and m + 1 < NP:
                    kf_p[m + 1][c, 0:8, :] = blk[rb - 8:, :]
                for rr in range(r, r + rb, 8):
                    ks = kf_p[m][c, 8 + rr:16 + rr, :] * taps[0]
                    for j in range(1, KS):
                        ks = ks + kf_p[m][c, 8 + rr - j:16 + rr - j, :] * taps[j]
                    u_p[m][c, rr:rr + 8, :] = ks * v_v[m * PC + rr:m * PC + rr + 8, cs].astype(F32)
                wrote(u_p[m], LAG_V)
            return f
        return [unit(c, r) for r in range(0, PC, rb) for c in range(NC)]

    def ht_prep(m):
        def unit(c, j):
            def f(tok):
                blk = h_v[m, c * 128:(c + 1) * 128, j * 128:(j + 1) * 128].astype(F32)
                tb = link(blk, tok).T
                if m == 0 and j == 0:
                    row0 = jax.lax.broadcasted_iota(jnp.int32, (8, 128), 0) == 0
                    dvec = dv_v[c * 128:(c + 1) * 128].astype(F32).reshape(1, 128)
                    tb = jnp.concatenate([tb[0:8] + jnp.where(row0, dvec, 0.0), tb[8:]], axis=0)
                ht_p[m][c, j * 128:(j + 1) * 128, :] = tb
                wrote(ht_p[m], LAG_V)
            return f
        return [unit(c, j) for c in range(NC) for j in range(PC // 128)]

    def spectral_unit(m, c, r, tok):
        us = slice(c * 128, (c + 1) * 128)
        hs = slice(D + c * 128, D + (c + 1) * 128)

        def ld(ref, k, ls):
            return ref[k, r:r + 8, ls], ref[k, 128 + r:128 + r + 8, ls]

        zu = [ld(z_p[m], k, us) for k in range(4)]
        zh = [ld(z_p[m], k, hs) for k in range(4)]
        for k in (0, 1):
            zu[k] = (link(zu[k][0], tok), link(zu[k][1], tok))
        for k in ((0, 1) if m == 0 else range(4)):
            zh[k] = (link(zh[k][0], tok), link(zh[k][1], tok))
        if m > 0:
            hp = [ld(z_p[m - 1], k, hs) for k in range(4)]
            if r < 64:
                zh = [(zh[k][0] - hp[k][1], zh[k][1] + hp[k][0]) for k in range(4)]
            else:
                zh = [(zh[k][0] + hp[k][1], zh[k][1] - hp[k][0]) for k in range(4)]
        um = _fft4(zu)
        gm = _fft4(zh)
        if m < NP - 1:
            for k in range(4):
                z_p[m][k, r:r + 8, us] = um[k][0]
                z_p[m][k, 128 + r:128 + r + 8, us] = um[k][1]
                gg_p[m][k, r:r + 8, us] = gm[k][0]
                gg_p[m][k, 128 + r:128 + r + 8, us] = gm[k][1]
            wrote(z_p[m], LAG_V)
            wrote(gg_p[m], LAG_V)
        ys = []
        prev = tok
        for k in range(4):
            re = im = None
            for b in range(m, -1, -1):
                ur, ui = um[k] if b == m else ld(z_p[b], k, us)
                gr, gi = gm[k] if b == 0 else ld(gg_p[m - b], k, us)
                if 0 < b < m:
                    ur, ui = link(ur, prev), link(ui, prev)
                pr = ur * gr - ui * gi
                pi = ur * gi + ui * gr
                re = pr if re is None else re + pr
                im = pi if im is None else im + pi
            ys.append((re, im))
            prev = re
        vs = _ifft4(ys)
        for s2 in range(4):
            vv_p[m][s2, r:r + 8, us] = _pk2(vs[s2][0], vs[s2][1])
        wrote(vv_p[m], LAG_V)

    def spectral(m):
        return [functools.partial(spectral_unit, m, c, r)
                for c in range(NC) for r in range(0, 128, 8)]

    out_cps = []

    def final(i):
        m = TSTART[i] // PC

        def unit(r):
            def f(tok):
                g0 = TSTART[i] + r
                pr = g0 - m * PC
                qf = [link(x_v[g0:g0 + 8, c * 128:(c + 1) * 128].astype(F32), tok)
                      for c in range(NC)]
                z = _tree([qf[c] * bc_s[c] for c in range(NC)], _add)
                zs = jnp.sum(z, axis=1, keepdims=True)
                g = _recip(1.0 + jnp.exp2(jnp.clip(zs * (-LOG2E), -126.0, 126.0)))
                rb = r - r % 16 + (r % 16) // 8
                for c in range(NC):
                    a = qf[c] * y_p[m][c, pr:pr + 8, :]
                    b = b_t[i][c, pl.ds(rb, 8, stride=2), :]
                    res = b + g * (a - b)
                    out_s[g0:g0 + 8, c * 128:(c + 1) * 128] = res.astype(BF16)
                st8["pend"].setdefault(due_step(LAG_FN), []).append(res)
                piece = TSIZES[i] // 2 if i == NT - 1 else TSIZES[i]
                if (r + 8) % piece == 0:
                    g1 = g0 + 8 - piece
                    out_cps.append(dma(out_s.at[pl.ds(g1, piece), :],
                                       out_hbm.at[pl.ds(g1, piece), :]))
            return f
        return [unit(r) for r in range(0, TSIZES[i], 8)]

    mtasks = {"P": proj, "O": outp, "F": fwd, "I": inv, "Pq": lambda n: proj(n, (0,)),
              "Pk": lambda n: proj(n, (1,)), "Pv": lambda n: proj(n, (2,))}
    vtasks = {"AT": attn, "A": spectral, "KV": kv_prep, "HT": ht_prep, "FN": final,
              "PW": prep_w, "PWO": prep_wo}
    vcache = {}

    def vunit(name, j):
        if name not in vcache:
            base, n = _split(name)
            vcache[name] = vtasks[base](n)
        return vcache[name][j]

    def run_plan(plan):
        steps = []
        for mname, units in plan:
            base, n = _split(mname)
            dots = mtasks[base](n)
            total, t0 = sum(d for d, _ in dots), 0
            for d, f in dots:
                steps.append((d, f, [(v, j, (fr * total - t0) / d) for v, j, fr in units
                                     if t0 <= fr * total < t0 + d]))
                t0 += d
        starts, t = [], 0
        for d, _, _ in steps:
            starts.append(t)
            t += d
        st8["starts"], st8["step"], st8["pend"], st8["dirty"] = starts + [t], 0, {}, {}
        for d, f, units in steps:
            toks = slices(f())
            for v, j, fr in units:
                vunit(v, j)(toks[int(fr * len(toks))])
            end_step()

    def spread(vname, lo, hi):
        return [(vname, j, SPAN * (j - lo) / (hi - lo)) for j in range(lo, hi)]

    for ref in o_t + bq_t + bk_t + bv_t + b_t + u_p + ht_p + y_p + z_p + gg_p + vv_p:
        for k in range(ref.shape[0]):
            ref[k, 0:8, 0:128] = jnp.zeros((8, 128), ref.dtype)
    for c in range(NC):
        bk_t[0][c, 0:HALO, :] = jnp.zeros((HALO, 128), F32)
        bv_t[0][c, 0:HALO, :] = jnp.zeros((HALO, 128), F32)
        kf_p[0][c, 0:8, :] = jnp.zeros((8, 128), F32)

    wait("z0 wq0")
    st8["mask"] = z0_v[...] != 0
    for rc in range(NC):
        if rc:
            wait("wq%d" % rc)
        vunit("PW0", rc)(None)
    wait("x0")
    run_plan([("Pq0", [])])
    wait("wk x1")
    issue_rest()
    run_plan([("Pq1", spread("PW1", 0, NC))])
    wait("wv")
    run_plan([("Pk0", spread("PW2", 0, NC)), ("Pv0", []),
              ("Pk1", spread("AT0", 0, 16)), ("Pv1", spread("AT0", 16, 32))])
    for k, (wset, plan) in enumerate(_make_plan(M_ORDER, V_PRIO)):
        wait(wset)
        if k == 0:
            for c in range(NC):
                cs = slice(c * 128, (c + 1) * 128)
                bc_s[c] = jnp.broadcast_to(gw_v[cs].astype(F32).reshape(1, 128), (8, 128))
                for j in range(KS):
                    bc_s[(1 + j) * NC + c] = jnp.broadcast_to(sk_v[j:j + 1, cs].astype(F32), (8, 128))
        run_plan(plan)
    for c_ in out_cps:
        c_.wait()


@jax.jit
def pallas_gated_mix__ssm_conv_h3__sliding_local_dilated__prompt_kernel(
    A_q: jax.Array,
    A_k: jax.Array,
    A_v: jax.Array,
    A_shift_k: jax.Array,
    A_ssm_k: jax.Array,
    A_ssm_D: jax.Array,
    B_x: jax.Array,
    B_wqkv: jax.Array,
    B_wo: jax.Array,
    gate_w: jax.Array,
):
    f_np, g_np = _dft_tables()
    vm = pltpu.VMEM
    scratch = [
        vm((S, D), BF16),
        vm((S, D), BF16),
        vm((KS, D), BF16),
        vm((NP, D, PC), BF16),
        vm((D,), BF16),
        vm((S, D), BF16),
        vm((3, D, D), BF16),
        vm((D, D), BF16),
        vm((D,), BF16),
        vm((4, 128, 128), U32),
        vm((4, 64, 256), U32),
        vm((8, 128), jnp.int32),
        vm((3 * D // 2, D), U32),
        vm((D // 2, D), U32),
        vm((4, NC, D, 128), F32),
        vm(((1 + KS) * NC, 8, 128), F32),
        vm((S, D), BF16),
        pltpu.SemaphoreType.DMA((48,)),
    ]
    scratch += [vm((T // 2, D), U32)] * NT
    scratch += [vm((2, T // 2, D), U32)] * NT
    scratch += [vm((NC, T, 128), F32)] * NT
    scratch += [vm((NC, T + HALO, 128), F32)] * NT
    scratch += [vm((NC, T + HALO, 128), F32)] * NT
    scratch += [vm((NC, T, 128), F32)] * NT
    scratch += [vm((NC, PC + 8, 128), F32)] * NP
    scratch += [vm((NC, PC, 128), F32)] * NP
    scratch += [vm((NC, PC, 128), F32)] * NP
    scratch += [vm((4, 64, 2 * D), U32)] * NP
    scratch += [vm((4, 256, 2 * D), F32)] * NP
    scratch += [vm((4, 256, D), F32)] * NP
    scratch += [vm((4, 128, D), U32)] * NP
    scratch += [vm((NC, PC, 128), F32)] * NP
    out = pl.pallas_call(
        _kernel,
        out_shape=jax.ShapeDtypeStruct((S, D), BF16),
        in_specs=[pl.BlockSpec(memory_space=pl.ANY)] * 12
        + [pl.BlockSpec(memory_space=pltpu.SMEM)],
        out_specs=pl.BlockSpec(memory_space=pl.ANY),
        scratch_shapes=scratch,
        compiler_params=pltpu.CompilerParams(vmem_limit_bytes=126 * 1024 * 1024),
    )(A_q.reshape(S, D), A_k.reshape(S, D), A_v.reshape(S, D), A_shift_k.T, A_ssm_k, A_ssm_D,
      B_wqkv, B_wo, gate_w, jnp.asarray(_pack_table(f_np)), jnp.asarray(_pack_table(g_np)),
      jnp.asarray(np.zeros((8, 128), np.int32)), jnp.asarray(np.zeros((1,), np.int32)))
    return out.reshape(1, S, D)
```
